```python
import os as _os
_os.environ.setdefault("JAX_PLATFORMS", "cpu")
import jax
import jax.numpy as jnp

def _softmax(x, axis=-1):
    return jax.nn.softmax(x, axis=axis)
def _gelu(x):
    return jax.nn.gelu(x, approximate=True)
def _silu(x):
    return jax.nn.silu(x)
def _sigmoid(x):
    return jax.nn.sigmoid(x)
def _layernorm(x, axis=-1, eps=1e-5):
    m = jnp.mean(x, axis=axis, keepdims=True)
    v = jnp.var(x, axis=axis, keepdims=True)
    return (x - m) / jnp.sqrt(v + eps)
def _scatter_add(tgt, idx, src, axis=0):
    return tgt.at[idx].add(src)
def _segment_sum(src, seg, n):
    return jax.ops.segment_sum(src, seg, n)
class _Rng:
    def __init__(self, key):
        self._k = key
    def _next(self):
        self._k, sub = jax.random.split(self._k)
        return sub
    def normal(self, shape):
        return jax.random.normal(self._next(), shape, dtype=jnp.bfloat16)
    def randint(self, lo, hi, shape):
        return jax.random.randint(self._next(), shape, lo, hi, dtype=jnp.int32)
    def uniform(self, shape, lo=0.0, hi=1.0):
        return jax.random.uniform(self._next(), shape, jnp.bfloat16, lo, hi)
    def permutation(self, n):
        return jax.random.permutation(self._next(), n)


kernel_name = 'gated_mix__linear_attn_block__mixer_s_mlp__prompt'

def setup_inputs():
    _rng = _Rng(jax.random.key(int.from_bytes(__import__("os").urandom(4), "little")))
    _w = (lambda a: (lambda t: t.astype(jnp.bfloat16) if jnp.issubdtype(t.dtype, jnp.floating) else t)(jnp.asarray(a)))
    def _A_setup():
        B, S, D = 1, 2048, 640
        return {
            "x": _w((lambda *s: _rng.normal(s) * 0.05)(B, S, D)),
            "wqkv": _w((lambda *s: _rng.normal(s) * 0.8)(D, 3 * D)),
            "wo": _w((lambda *s: _rng.normal(s) * 0.1)(D, D)),
        }
    _A_in = _A_setup()

    def _B_setup():
        B, S, D, F = 1, 2048, 640, 1728
        return {
            "x":  _w((lambda *s: _rng.normal(s) * 0.05)(B, S, D)),
            "w1": _w((lambda *s: _rng.normal(s) * 0.2)(D, D) * (D ** -0.5)),
            "w2": _w((lambda *s: _rng.normal(s) * 0.2)(D, D) * (D ** -0.5)),
            "w3": _w((lambda *s: _rng.normal(s) * 0.2)(D, F) * (D ** -0.5)),
            "w4": _w((lambda *s: _rng.normal(s) * 0.2)(F, D) * (F ** -0.5)),
        }
    _B_in = _B_setup()

    return {
        "A_x": _A_in["x"],
        "A_wqkv": _A_in["wqkv"],
        "A_wo": _A_in["wo"],
        "B_x": _B_in["x"],
        "B_w1": _B_in["w1"],
        "B_w2": _B_in["w2"],
        "B_w3": _B_in["w3"],
        "B_w4": _B_in["w4"],
        "gate_w": _w((lambda *s: _rng.normal(s) * 0.05)(640) * 16.0),
    }

def reference(A_x, A_wqkv, A_wo, B_x, B_w1, B_w2, B_w3, B_w4, gate_w):
    def _A_ref(x, wqkv, wo):
        B, S, D = x.shape
        H = 32; Dh = D // H
        qkv = (lambda x, *d: x.transpose(*d))((x @ wqkv).reshape(B, S, 3, H, Dh), 2, 0, 3, 1, 4)
        q, k, v = qkv[0], qkv[1], qkv[2]
        phi = lambda t: jnp.where(t > 0, t + 1, jnp.exp(t)) + 1e-6
        pq, pk = phi(q), phi(k)
        kv = jnp.einsum("bhsd,bhse->bhde", pk, v)
        z = jnp.einsum("bhsd->bhd", pk)
        num = jnp.einsum("bhqd,bhde->bhqe", pq, kv)
        den = jnp.einsum("bhqd,bhd->bhq", pq, z)[..., None] + 1e-6
        o = num / den
        return (lambda x, *d: x.transpose(*d))(o, 0, 2, 1, 3).reshape(B, S, D) @ wo

    def _B_ref(x, w1, w2, w3, w4):
        B, S, D = x.shape
        h = _gelu(_layernorm(x, axis=-1) @ w1)
        c = D // 4
        g0 = jnp.pad(h[:, :, 0*c:1*c], ((0, 0), (1, 0), (0, 0)))[:, :S, :]
        g1 = jnp.pad(h[:, :, 1*c:2*c], ((0, 0), (0, 1), (0, 0)))[:, 1:, :]
        g2 = jnp.pad(h[:, :, 2*c:3*c], ((0, 0), (2, 0), (0, 0)))[:, :S, :]
        g3 = jnp.pad(h[:, :, 3*c:   ], ((0, 0), (0, 2), (0, 0)))[:, 2:, :]
        hs = jnp.concatenate([g0, g1, g2, g3], axis=-1) @ w2
        x1 = x + hs
        h2 = _gelu(_layernorm(x1, axis=-1) @ w3) @ w4
        return x1 + h2

    x = A_x
    g = _sigmoid((x * gate_w).sum(-1, keepdims=True))
    a = _A_ref(x, A_wqkv, A_wo)
    b = _B_ref(x, B_w1, B_w2, B_w3, B_w4)
    return g * a + (1 - g) * b
```

```python
import contextlib
import jax
import jax.numpy as jnp
from jax import lax
from jax.experimental import pallas as pl
from jax.experimental.pallas import tpu as pltpu

S, D, F, H, DH = 2048, 640, 1728, 32, 20
LT = D // 128
FM = 1664
KV_ROWS = ((0, 144), (112, 272), (240, 400), (368, 528), (496, 640))
PAD = 8
F32 = jnp.float32
BF16 = jnp.bfloat16

NN = (((1,), (0,)), ((), ()))
NT_ = (((1,), (1,)), ((), ()))


def _dot(a, b, dims=NN):
    return lax.dot_general(a, b, dims, preferred_element_type=F32)


def _phi(t):
    return jnp.where(t > 0, t + 1.0, jnp.exp(t)) + 1e-6


def _gelu(x):
    c = 0.7978845608028654
    inner = x * (c + (c * 0.044715) * (x * x))
    hx = 0.5 * x
    return hx + hx * jnp.tanh(inner)


def _ln(x):
    m = jnp.mean(x, axis=-1, keepdims=True)
    xc = x - m
    v = jnp.mean(xc * xc, axis=-1, keepdims=True)
    return xc * lax.rsqrt(v + 1e-5)


def make(TF=256, TD=512, TM=(128,), TL=(320, 320), half=True, scopes=False, orderL=0, orderM=0, dorder='x0 gw k0 | k1 k2 w1 x1 xl wq'):
    N1 = (S - 2 * TF) // TD
    assert 2 * TF + N1 * TD == S
    RM = sum(TM)
    BL = sum(TL)
    N2 = (S - RM) // BL
    assert RM + N2 * BL == S
    TMAX = max(max(TM), max(TL))
    NSL = max(len(TM), len(TL))
    FH = F // 2

    def scope(name):
        return jax.named_scope(name) if scopes else contextlib.nullcontext()

    def kernel(ax_hbm, wqkv_hbm, wo_hbm, w1_hbm, w2_hbm, w3_hbm, w4_hbm, gw_hbm, out_hbm,
               ax, wq, wk, wv, wo, w1, w2, w3, w4, gw, ob,
               wkT, wqTp, tmp, hbuf, gacc, zacc, Mp, zrow,
               xn1, pqs, pqn, hsb, x1s, xns, gas, gus, gts,
               sx, sw, so):
        def xcopy(r0, n, i):
            return pltpu.make_async_copy(ax_hbm.at[0, pl.ds(r0, n), :], ax.at[pl.ds(r0, n), :], sx.at[i])

        def xloop(t):
            return xcopy(2 * TF + t * TD, TD, 2 + t)

        wcopies = {
            'w1': pltpu.make_async_copy(w1_hbm, w1, sw.at[0]),
            'wv': pltpu.make_async_copy(wqkv_hbm.at[:, pl.ds(2 * D, D)], wv, sw.at[2]),
            'wq': pltpu.make_async_copy(wqkv_hbm.at[:, pl.ds(0, D)], wq, sw.at[3]),
            'wo': pltpu.make_async_copy(wo_hbm, wo, sw.at[4]),
            'w2': pltpu.make_async_copy(w2_hbm, w2, sw.at[5]),
            'w3a': pltpu.make_async_copy(w3_hbm.at[pl.ds(0, FH), :], w3.at[pl.ds(0, FH), :], sw.at[6]),
            'w3b': pltpu.make_async_copy(w3_hbm.at[pl.ds(FH, FH), :], w3.at[pl.ds(FH, FH), :], sw.at[7]),
            'w4a': pltpu.make_async_copy(w4_hbm.at[pl.ds(0, FH), :], w4.at[pl.ds(0, FH), :], sw.at[8]),
            'w4b': pltpu.make_async_copy(w4_hbm.at[pl.ds(FH, FH), :], w4.at[pl.ds(FH, FH), :], sw.at[9]),
            'gw': pltpu.make_async_copy(gw_hbm, gw, sw.at[10]),
        }
        late = ['wv', 'w2', 'wo', 'w3a', 'w3b', 'w4a', 'w4b']
        groups = [late[(i * len(late)) // N1:((i + 1) * len(late)) // N1] for i in range(N1)]

        def al(r, m):
            return r if isinstance(r, int) else pl.multiple_of(r, m)

        def ln1(r0, n, o=0):
            gwf = gw[...].astype(F32).reshape(1, D)
            x = ax[pl.ds(al(r0, 16), n), :].astype(F32)
            xn1[o:o + n, :] = _ln(x).astype(BF16)
            lg = jnp.sum(x * gwf, axis=-1, keepdims=True)
            g = 0.5 * jnp.tanh(0.5 * lg) + 0.5
            gts[pl.ds(al(r0, 16), n), :] = jnp.broadcast_to(g, (n, 128))

        def h_dot(r0, n, o=0):
            h = _gelu(_dot(xn1[o:o + n, :], w1[...]))
            for j in range(LT):
                hbuf[j, pl.ds(al(r0 + PAD, 8), n), :] = h[:, 128 * j:128 * (j + 1)]

        def k_dot(r0, n, split=False):
            xa = ax[pl.ds(al(r0, 16), n), :]
            if split:
                pk = jnp.concatenate([_phi(_dot(wkT[0:320, :], xa, NT_)), _phi(_dot(wkT[320:640, :], xa, NT_))], axis=0)
            else:
                pk = _phi(_dot(wkT[...], xa, NT_))
            zs = pk[:, 0:128]
            for j in range(1, n // 128):
                zs = zs + pk[:, 128 * j:128 * (j + 1)]
            return pk.astype(BF16), zs

        def g_dot(r0, n, pkb, first, split=False):
            xa = ax[pl.ds(al(r0, 16), n), :]
            for a, b in (((0, 320), (320, 640)) if split else ((0, 640),)):
                if first:
                    gacc[a:b, :] = _dot(pkb[a:b, :], xa)
                else:
                    gacc[a:b, :] += _dot(pkb[a:b, :], xa)

        def wq_slice(lt):
            rows = wq[pl.ds(al(lt * 128, 128), 128), :]
            tmp[0] = rows.T.astype(F32)
            for j in range(LT):
                for c in range(4):
                    wqTp[lt, pl.ds(128 * j + 32 * c, 32), :] = (
                        tmp[0, pl.ds(4 * j + c, 32, stride=DH), :].astype(BF16))

        WKC = ((0, 256), (256, 512), (512, 640))
        wkc = [pltpu.make_async_copy(wqkv_hbm.at[pl.ds(a, b - a), pl.ds(D, D)], wk.at[pl.ds(a, b - a), :], sw.at[11 + i])
               for i, (a, b) in enumerate(WKC)]

        starts = {
            'gw': lambda: wcopies['gw'].start(), 'x0': lambda: xcopy(0, TF, 0).start(),
            'k0': lambda: wkc[0].start(), 'k1': lambda: wkc[1].start(), 'k2': lambda: wkc[2].start(),
            'w1': lambda: wcopies['w1'].start(), 'x1': lambda: xcopy(TF, TF, 1).start(),
            'xl': lambda: xloop(0).start(), 'wq': lambda: wcopies['wq'].start()}
        pre, post = dorder.split('|')
        for n in pre.split():
            starts[n]()

        with scope('p1first'):
            for j in range(LT):
                hbuf[j, 0:PAD, :] = jnp.zeros((PAD, 128), F32)
                hbuf[j, PAD + S:PAD + S + PAD, :] = jnp.zeros((PAD, 128), F32)
            with scope('w_x0'):
                xcopy(0, TF, 0).wait()
            for n in post.split():
                starts[n]()
            with scope('w_gw'):
                wcopies['gw'].wait()
            with scope('ln0'):
                ln1(0, TF)
            for ci, (c, (a, b)) in enumerate(zip(wkc, WKC)):
                with scope(f'w_wk{ci}'):
                    c.wait()
                with scope(f'tr{ci}'):
                    wkT[:, a:b] = wk[a:b, :].T
            with scope('kdot0'):
                pkb, zs = k_dot(0, TF, split=True)
            with scope('w_w1'):
                wcopies['w1'].wait()
                xcopy(TF, TF, 1).wait()
            with scope('rest'):
                h_dot(0, TF)
                pkb1, zs1 = k_dot(TF, TF)
                ln1(TF, TF, TF)
                zacc[...] = zs + zs1
                g_dot(0, TF, pkb, True)
                h_dot(TF, TF, TF)
                g_dot(TF, TF, pkb1, False, split=True)

        def phase1(t, carry):
            with scope('p1body'):
                @pl.when(t + 1 < N1)
                def _():
                    xloop(t + 1).start()
                for i in range(N1):
                    if groups[i]:
                        @pl.when(t == i)
                        def _(i=i):
                            for n in groups[i]:
                                wcopies[n].start()

                @pl.when(t == 0)
                def _():
                    wcopies['wq'].wait()
                xloop(t).wait()
                r0 = al(2 * TF + t * TD, 128)
                pkb, zs = k_dot(r0, TD)
                ln1(r0, TD)
                h_dot(r0, TD)
                zacc[...] += zs
                g_dot(r0, TD, pkb, False)
                nsl = -(-LT // N1)
                for u in range(nsl):
                    wq_slice(jnp.minimum(t * nsl + u, LT - 1))
            return carry

        lax.fori_loop(0, N1, phase1, 0)

        def kv_dots():
            outs = []
            for j in range(LT):
                a, b = KV_ROWS[j]
                kvj = _dot(gacc[a:b, :].astype(BF16), wv[:, 128 * j:128 * (j + 1)])
                rh = (lax.broadcasted_iota(jnp.int32, (b - a, 128), 0) + a) // DH
                ch = (lax.broadcasted_iota(jnp.int32, (b - a, 128), 1) + 128 * j) // DH
                outs.append(jnp.where(rh == ch, kvj, 0.0).astype(BF16))
            return outs

        def m_dots(kvms):
            carry = None
            for j in range(LT):
                a, b = KV_ROWS[j]
                part = _dot(kvms[j], wo[128 * j:128 * (j + 1), :])
                lo = 0
                if carry is not None:
                    head = part[0:32, :] + carry
                    for lt in range(LT):
                        tmp[lt, a:a + 32, :] = head[:, 128 * lt:128 * (lt + 1)]
                    lo = 32
                hi = (b - a) - (32 if j + 1 < LT else 0)
                for lt in range(LT):
                    tmp[lt, a + lo:a + hi, :] = part[lo:hi, 128 * lt:128 * (lt + 1)]
                carry = part[hi:b - a, :] if j + 1 < LT else None
            for j in range(LT):
                for c in range(4):
                    for lt in range(LT):
                        Mp[pl.ds(128 * j + 32 * c, 32), pl.ds(128 * lt, 128)] = (
                            tmp[lt, pl.ds(4 * j + c, 32, stride=DH), :].astype(BF16))

        def z_setup():
            for j in range(LT):
                zp = jnp.concatenate([zacc[pl.ds(4 * j + c, 32, stride=DH), :] for c in range(4)], axis=0)
                zrow[:, 128 * j:128 * (j + 1)] = jnp.sum(zp.T, axis=0, keepdims=True)

        def q_dot(s, r0, T):
            xa = ax[pl.ds(al(r0, 16), T), :]
            wt = jnp.concatenate([wqTp[lt] for lt in range(LT)], axis=1)
            pqs[s, 0:T] = _phi(_dot(xa, wt, NT_))

        def nrm(s, T):
            z = zrow[...]
            pq = pqs[s, 0:T]
            sm = pq[:, 0:128] * z[:, 0:128]
            for j in range(1, LT):
                sm = sm + pq[:, 128 * j:128 * (j + 1)] * z[:, 128 * j:128 * (j + 1)]
            sm = sm + pltpu.roll(sm, 64, 1)
            sm = sm + pltpu.roll(sm, 32, 1)
            rr = 1.0 / (sm + 1e-6)
            pqn[s, 0:T] = jnp.concatenate(
                [pq[:, 128 * j:128 * (j + 1)] * rr for j in range(LT)], axis=1).astype(BF16)

        def hs_asm(s, r0, T):
            def hl(j, sh):
                return hbuf[j, pl.ds(r0 + PAD - sh, T), :]
            lane = lax.broadcasted_iota(jnp.int32, (T, 128), 1)
            hsb[s, 0:T] = jnp.concatenate([
                hl(0, 1),
                jnp.where(lane < 32, hl(1, 1), hl(1, -1)),
                jnp.where(lane < 64, hl(2, -1), hl(2, 2)),
                jnp.where(lane < 96, hl(3, 2), hl(3, -2)),
                hl(4, -2)], axis=1).astype(BF16)

        def w2_dot(s, r0, T):
            xa = ax[pl.ds(al(r0, 16), T), :]
            x1s[s, 0:T] = xa.astype(F32) + _dot(hsb[s, 0:T], w2[...])

        def m_dot(s, r0, T):
            a = _dot(pqn[s, 0:T], Mp[...])
            g = gts[pl.ds(al(r0, 16), T), :]
            for j in range(LT):
                sl = slice(128 * j, 128 * (j + 1))
                gas[s, 0:T, sl] = g * a[:, sl] + (1.0 - g) * x1s[s, 0:T, sl]

        def ln2(s, T):
            xns[s, 0:T] = _ln(x1s[s, 0:T]).astype(BF16)

        def w3_dot(s, T):
            xn = xns[s, 0:T]
            if half:
                gus[s, 0:T, 0:FM] = _gelu(_dot(xn, w3[0:FM, :], NT_)).astype(BF16)
                ut = _dot(w3[FM:F, :], xn, NT_)
                gus[s, 0:T, FM:F] = _gelu(ut).T.astype(BF16)
            else:
                gus[s, 0:T, 0:F] = _gelu(_dot(xn, w3[...], NT_)).astype(BF16)

        def ocopy(r0, T, i):
            return pltpu.make_async_copy(ob.at[pl.ds(r0, T), :], out_hbm.at[0, pl.ds(r0, T), :], so.at[i])

        def w4_dot(s, r0, T, i):
            h2 = _dot(gus[s, 0:T, 0:F], w4[...])
            g = gts[pl.ds(al(r0, 16), T), :]
            for j in range(LT):
                sl = slice(128 * j, 128 * (j + 1))
                ob[pl.ds(al(r0, 16), T), sl] = (gas[s, 0:T, sl] + (1.0 - g) * h2[:, sl]).astype(BF16)
            ocopy(al(r0, 16), T, i).start()

        def body_m():
            if len(TM) == 1:
                T = TM[0]
                q_dot(0, 0, T)
                kvm = kv_dots()
                hs_asm(0, 0, T)
                z_setup()
                w2_dot(0, 0, T)
                m_dots(kvm)
                ln2(0, T)
                nrm(0, T)
                w3_dot(0, T)
                m_dot(0, 0, T)
                w4_dot(0, 0, T, 0)
            else:
                TA, TB = TM
                A, B = 0, TA
                q_dot(0, A, TA)
                kvm = kv_dots()
                hs_asm(0, A, TA)
                z_setup()
                w2_dot(0, A, TA)
                m_dots(kvm)
                hs_asm(1, B, TB)
                q_dot(1, B, TB)
                ln2(0, TA)
                w2_dot(1, B, TB)
                nrm(0, TA)
                w3_dot(0, TA)
                m_dot(0, A, TA)
                nrm(1, TB)
                ln2(1, TB)
                m_dot(1, B, TB)
                w4_dot(0, A, TA, 0)
                w3_dot(1, TB)
                w4_dot(1, B, TB, 1)

        def body_l(t):
            base = RM + t * BL
            i0 = len(TM) + t * len(TL)
            if len(TL) == 1:
                T = TL[0]
                r0 = al(base, 16)
                q_dot(0, r0, T)
                hs_asm(0, r0, T)
                w2_dot(0, r0, T)
                nrm(0, T)
                m_dot(0, r0, T)
                ln2(0, T)
                w3_dot(0, T)
                w4_dot(0, r0, T, i0)
            else:
                TA, TB = TL
                A, B = al(base, 16), al(base + TA, 16)
                if orderL == 0:
                    q_dot(0, A, TA)
                    hs_asm(0, A, TA)
                    w2_dot(0, A, TA)
                    q_dot(1, B, TB)
                    nrm(0, TA)
                    hs_asm(1, B, TB)
                    m_dot(0, A, TA)
                    w2_dot(1, B, TB)
                    ln2(0, TA)
                    w3_dot(0, TA)
                    nrm(1, TB)
                    m_dot(1, B, TB)
                    ln2(1, TB)
                    w4_dot(0, A, TA, i0)
                    w3_dot(1, TB)
                    w4_dot(1, B, TB, i0 + 1)
                elif orderL == 1:
                    q_dot(0, A, TA)
                    hs_asm(0, A, TA)
                    w2_dot(0, A, TA)
                    q_dot(1, B, TB)
                    hs_asm(1, B, TB)
                    w2_dot(1, B, TB)
                    nrm(0, TA)
                    m_dot(0, A, TA)
                    ln2(0, TA)
                    w3_dot(0, TA)
                    nrm(1, TB)
                    m_dot(1, B, TB)
                    ln2(1, TB)
                    w4_dot(0, A, TA, i0)
                    w3_dot(1, TB)
                    w4_dot(1, B, TB, i0 + 1)

        with scope('pm'):
            for n in late:
                wcopies[n].wait()
            body_m()

        def phase2(t, carry):
            with scope('p2body'):
                body_l(t)
            return carry

        lax.fori_loop(0, N2, phase2, 0)
        with scope('fin'):
            r = 0
            i = 0
            for T in list(TM) + list(TL) * N2:
                ocopy(r, T, i).wait()
                r += T
                i += 1

    NOUT = len(TM) + N2 * len(TL)

    def fn(A_x, A_wqkv, A_wo, B_x, B_w1, B_w2, B_w3, B_w4, gate_w):
        anyspec = pl.BlockSpec(memory_space=pltpu.HBM)
        return pl.pallas_call(
            kernel,
            out_shape=jax.ShapeDtypeStruct((1, S, D), BF16),
            in_specs=[anyspec] * 8,
            out_specs=anyspec,
            scratch_shapes=[
                pltpu.VMEM((S, D), BF16),
                pltpu.VMEM((D, D), BF16), pltpu.VMEM((D, D), BF16), pltpu.VMEM((D, D), BF16),
                pltpu.VMEM((D, D), BF16), pltpu.VMEM((D, D), BF16), pltpu.VMEM((D, D), BF16),
                pltpu.VMEM((F, D), BF16), pltpu.VMEM((F, D), BF16),
                pltpu.VMEM((D,), BF16), pltpu.VMEM((S, D), BF16),
                pltpu.VMEM((D, D), BF16), pltpu.VMEM((LT, D, 128), BF16),
                pltpu.VMEM((LT, D, 128), F32),
                pltpu.VMEM((LT, S + 2 * PAD, 128), F32),
                pltpu.VMEM((D, D), F32),
                pltpu.VMEM((D, 128), F32),
                pltpu.VMEM((D, D), BF16),
                pltpu.VMEM((1, D), F32),
                pltpu.VMEM((max(TD, 2 * TF), D), BF16),
                pltpu.VMEM((NSL, TMAX, D), F32),
                pltpu.VMEM((NSL, TMAX, D), BF16),
                pltpu.VMEM((NSL, TMAX, D), BF16),
                pltpu.VMEM((NSL, TMAX, D), F32),
                pltpu.VMEM((NSL, TMAX, D), BF16),
                pltpu.VMEM((NSL, TMAX, D), F32),
                pltpu.VMEM((NSL, TMAX, 1792), BF16),
                pltpu.VMEM((S, 128), F32),
                pltpu.SemaphoreType.DMA((2 + N1,)),
                pltpu.SemaphoreType.DMA((14,)),
                pltpu.SemaphoreType.DMA((NOUT,)),
            ],
            compiler_params=pltpu.CompilerParams(vmem_limit_bytes=100 * 1024 * 1024),
            name='gm',
        )(A_x, A_wqkv, A_wo, B_w1, B_w2, B_w3.T, B_w4, gate_w)
    return fn


_impl = make(TM=(256,), TL=(256,))


@jax.jit
def pallas_gated_mix__linear_attn_block__mixer_s_mlp__prompt_kernel(A_x, A_wqkv, A_wo, B_x, B_w1, B_w2, B_w3, B_w4, gate_w):
    return _impl(A_x, A_wqkv, A_wo, B_x, B_w1, B_w2, B_w3, B_w4, gate_w)
```

```python
import contextlib
import jax
import jax.numpy as jnp
from jax import lax
from jax.experimental import pallas as pl
from jax.experimental.pallas import tpu as pltpu

S, D, F, H, DH = 2048, 640, 1728, 32, 20
LT = D // 128
FM = 1664
KV_ROWS = ((0, 144), (112, 272), (240, 400), (368, 528), (496, 640))
PAD = 8
F32 = jnp.float32
BF16 = jnp.bfloat16

NN = (((1,), (0,)), ((), ()))
NT_ = (((1,), (1,)), ((), ()))


def _dot(a, b, dims=NN):
    return lax.dot_general(a, b, dims, preferred_element_type=F32)


def _phi(t):
    return jnp.where(t > 0, t + 1.0, jnp.exp(t)) + 1e-6


def _gelu(x):
    c = 0.7978845608028654
    inner = x * (c + (c * 0.044715) * (x * x))
    hx = 0.5 * x
    return hx + hx * jnp.tanh(inner)


def _stats(x):
    m = jnp.mean(x, axis=-1, keepdims=True)
    xc = x - m
    v = jnp.mean(xc * xc, axis=-1, keepdims=True)
    return m, xc, lax.rsqrt(v + 1e-5)


def _ln(x):
    m, xc, rs = _stats(x)
    return xc * rs


def make(TF=256, N1=4, HR=368, TM=(256,), TL=(224, 224), scopes=False, KA=256, orderM=1, nobc=False, osplit=False, nosc=False, ln2out=False,
         dorder='x0 gw a0 | a1 x1 k0 x2 k1 k2 x3 r0 wq'):
    NF = 4
    TD = S // N1
    NL = N1 - 1
    RF = S - NL * HR
    T3 = RF - 3 * TF
    assert T3 > 0 and T3 % 16 == 0 and HR % 16 == 0 and TD % 128 == 0
    RM = sum(TM)
    BL = sum(TL)
    N2 = (S - RM) // BL
    assert RM + N2 * BL == S
    TMAX = max(max(TM), max(TL))
    NSL = max(len(TM), len(TL))
    FH = F // 2
    NOUT = len(TM) + N2 * len(TL)

    def scope(name):
        return jax.named_scope(name) if scopes else contextlib.nullcontext()

    def kernel(ax_hbm, wqkv_hbm, wo_hbm, w1_hbm, w2_hbm, w3_hbm, w4_hbm, gw_hbm, out_hbm,
               ax, wq, wk, wv, wo, w1, w2, w3, w4, gw, ob,
               wkT, wqTp, tmp, tmp2, hbuf, gacc, zacc, Mp, zrow,
               hacc, st0, c1s, c3s, pqs, pqn, hsb, x1s, xns, gas, gus, gts,
               sx, sw, so):
        def xcopy(r0, n, i):
            return pltpu.make_async_copy(ax_hbm.at[0, pl.ds(r0, n), :], ax.at[pl.ds(r0, n), :], sx.at[i])

        def xrest(t):
            return xcopy(RF + t * HR, HR, NF + t)

        def wcopy(n):
            return {
                'a0': lambda: pltpu.make_async_copy(w1_hbm.at[pl.ds(0, KA), :], w1.at[pl.ds(0, KA), :], sw.at[0]),
                'a1': lambda: pltpu.make_async_copy(w1_hbm.at[pl.ds(KA, D - KA), :], w1.at[pl.ds(KA, D - KA), :], sw.at[1]),
                'wv': lambda: pltpu.make_async_copy(wqkv_hbm.at[:, pl.ds(2 * D, D)], wv, sw.at[2]),
                'wq': lambda: pltpu.make_async_copy(wqkv_hbm.at[:, pl.ds(0, D)], wq, sw.at[3]),
                'wo': lambda: pltpu.make_async_copy(wo_hbm, wo, sw.at[4]),
                'w2': lambda: pltpu.make_async_copy(w2_hbm, w2, sw.at[5]),
                'w3a': lambda: pltpu.make_async_copy(w3_hbm.at[pl.ds(0, FH), :], w3.at[pl.ds(0, FH), :], sw.at[6]),
                'w3b': lambda: pltpu.make_async_copy(w3_hbm.at[pl.ds(FH, FH), :], w3.at[pl.ds(FH, FH), :], sw.at[7]),
                'w4a': lambda: pltpu.make_async_copy(w4_hbm.at[pl.ds(0, FH), :], w4.at[pl.ds(0, FH), :], sw.at[8]),
                'w4b': lambda: pltpu.make_async_copy(w4_hbm.at[pl.ds(FH, FH), :], w4.at[pl.ds(FH, FH), :], sw.at[9]),
                'gw': lambda: pltpu.make_async_copy(gw_hbm, gw, sw.at[10]),
                'k0': lambda: pltpu.make_async_copy(wqkv_hbm.at[pl.ds(0, 256), pl.ds(D, D)], wk.at[pl.ds(0, 256), :], sw.at[11]),
                'k1': lambda: pltpu.make_async_copy(wqkv_hbm.at[pl.ds(256, 256), pl.ds(D, D)], wk.at[pl.ds(256, 256), :], sw.at[12]),
                'k2': lambda: pltpu.make_async_copy(wqkv_hbm.at[pl.ds(512, 128), pl.ds(D, D)], wk.at[pl.ds(512, 128), :], sw.at[13]),
                'x0': lambda: xcopy(0, TF, 0),
                'x1': lambda: xcopy(TF, TF, 1),
                'x2': lambda: xcopy(2 * TF, TF, 2),
                'x3': lambda: xcopy(3 * TF, T3, 3),
                'r0': lambda: xrest(0),
            }[n]()

        late = ['wv', 'w2', 'wo', 'w3a', 'w3b', 'w4a', 'w4b']
        groups = [late[(i * len(late)) // NL:((i + 1) * len(late)) // NL] for i in range(NL)]

        def al(r, m):
            return r if isinstance(r, int) else pl.multiple_of(r, m)

        def h_epi(y, r0, n, pre=None):
            if pre is not None:
                rs, rm = st0[0], st0[1]
                c1 = pre
                for j in range(LT):
                    sl = slice(128 * j, 128 * (j + 1))
                    hbuf[j, pl.ds(al(r0 + PAD, 8), n), :] = _gelu(y[:, sl] * rs - rm * c1[:, sl])
                return
            x = ax[pl.ds(al(r0, 16), n), :].astype(F32)
            m, _, rs = _stats(x)
            h = _gelu(y * rs - (rs * m) * c1s[...])
            for j in range(LT):
                hbuf[j, pl.ds(al(r0 + PAD, 8), n), :] = h[:, 128 * j:128 * (j + 1)]

        def h_dot(r0, n):
            h_epi(_dot(ax[pl.ds(al(r0, 16), n), :], w1[...]), r0, n)

        def k_dot(r0, n):
            xa = ax[pl.ds(al(r0, 16), n), :]
            kk = _dot(wkT[...], xa, NT_)
            pk = _phi(kk[0:D, :])
            g = 0.5 * jnp.tanh(0.5 * kk[D:D + 1, :]) + 0.5
            gts[pl.ds(al(r0, 128), n), :] = jnp.broadcast_to(g, (128, n)).T
            zs = pk[:, 0:128]
            for j in range(1, n // 128):
                zs = zs + pk[:, 128 * j:128 * (j + 1)]
            return pk.astype(BF16), zs

        def g_dot(r0, n, pkb):
            xa = ax[pl.ds(al(r0, 16), n), :]
            gacc[...] += _dot(pkb, xa)

        def wq_slice(lt, buf, slot):
            rows = wq[pl.ds(lt * 128, 128), :]
            buf[slot] = rows.T.astype(F32)
            for j in range(LT):
                for c in range(4):
                    wqTp[lt, pl.ds(128 * j + 32 * c, 32), :] = (
                        buf[slot, pl.ds(4 * j + c, 32, stride=DH), :].astype(BF16))

        def transp(a, b):
            wkT[0:D, a:b] = wk[a:b, :].T

        pre, post = dorder.split('|')
        for n in pre.split():
            wcopy(n).start()

        with scope('p1first'):
            for j in range(LT):
                hbuf[j, 0:PAD, :] = jnp.zeros((PAD, 128), F32)
                hbuf[j, PAD + S:PAD + S + PAD, :] = jnp.zeros((PAD, 128), F32)
            ones = jnp.ones((16, D), BF16)
            with scope('w_x0'):
                wcopy('x0').wait()
            for n in post.split():
                wcopy(n).start()
            wcopy('gw').wait()
            with scope('st0'):
                m0, _, rs0 = _stats(ax[0:TF, :].astype(F32))
                st0[0] = jnp.broadcast_to(rs0, (TF, 128))
                st0[1] = jnp.broadcast_to(rs0 * m0, (TF, 128))
            with scope('w_a0'):
                wcopy('a0').wait()
            with scope('R1'):
                lhs = jnp.concatenate([ones[:, 0:KA], ax[0:TF, 0:KA]], axis=0)
                hacc[...] = _dot(lhs, w1[0:KA, :])
            with scope('w_a1'):
                wcopy('a1').wait()
            with scope('R2'):
                lhs = jnp.concatenate([ones[:, KA:D], ax[0:TF, KA:D]], axis=0)
                y = hacc[...] + _dot(lhs, w1[KA:D, :])
                c1s[...] = y[0:1, :]
                h_epi(y[16:16 + TF, :], 0, TF, pre=y[0:1, :])
            with scope('w_3'):
                wcopy('x1').wait()
            with scope('R3'):
                h_dot(TF, TF)
            with scope('w_4'):
                for n in ('k0', 'x2', 'k1', 'k2', 'x3'):
                    wcopy(n).wait()
            with scope('R4'):
                transp(0, 256)
                transp(256, 512)
                transp(512, 640)
                grow = lax.broadcasted_iota(jnp.int32, (16, D), 0)
                wkT[D:D + 16, :] = jnp.where(
                    grow == 0, jnp.broadcast_to(gw[...].astype(F32).reshape(1, D), (16, D)), 0.0).astype(BF16)
                h_dot(2 * TF, TF)
                pkb, zs = k_dot(0, TD)
                h_dot(3 * TF, T3)
                zacc[...] = zs
                gacc[...] = _dot(pkb, ax[0:TD, :])

        def phase1(t, carry):
            with scope('p1body'):
                @pl.when(t + 1 < NL)
                def _():
                    xrest(t + 1).start()
                for i in range(NL):
                    if groups[i]:
                        @pl.when(t == i)
                        def _(i=i):
                            for n in groups[i]:
                                wcopy(n).start()
                xrest(t).wait()
                r0 = al((t + 1) * TD, 128)
                pkb, zs = k_dot(r0, TD)
                h_dot(al(RF + t * HR, 16), HR)
                zacc[...] += zs
                g_dot(r0, TD, pkb)
            return carry

        lax.fori_loop(0, NL, phase1, 0)

        def kv_dots():
            outs = []
            for j in range(LT):
                a, b = KV_ROWS[j]
                kvj = _dot(gacc[a:b, :].astype(BF16), wv[:, 128 * j:128 * (j + 1)])
                rh = (lax.broadcasted_iota(jnp.int32, (b - a, 128), 0) + a) // DH
                ch = (lax.broadcasted_iota(jnp.int32, (b - a, 128), 1) + 128 * j) // DH
                outs.append(jnp.where(rh == ch, kvj, 0.0).astype(BF16))
            return outs

        def m_dots(kvms):
            carry = None
            for j in range(LT):
                a, b = KV_ROWS[j]
                part = _dot(kvms[j], wo[128 * j:128 * (j + 1), :])
                lo = 0
                if carry is not None:
                    head = part[0:32, :] + carry
                    for lt in range(LT):
                        tmp[lt, a:a + 32, :] = head[:, 128 * lt:128 * (lt + 1)]
                    lo = 32
                hi = (b - a) - (32 if j + 1 < LT else 0)
                for lt in range(LT):
                    tmp[lt, a + lo:a + hi, :] = part[lo:hi, 128 * lt:128 * (lt + 1)]
                carry = part[hi:b - a, :] if j + 1 < LT else None
            for j in range(LT):
                for c in range(4):
                    for lt in range(LT):
                        Mp[pl.ds(128 * j + 32 * c, 32), pl.ds(128 * lt, 128)] = (
                            tmp[lt, pl.ds(4 * j + c, 32, stride=DH), :].astype(BF16))

        def z_setup():
            for j in range(LT):
                zp = jnp.concatenate([zacc[pl.ds(4 * j + c, 32, stride=DH), :] for c in range(4)], axis=0)
                zrow[:, 128 * j:128 * (j + 1)] = jnp.sum(zp.T, axis=0, keepdims=True)

        def q_dot(s, r0, T):
            xa = ax[pl.ds(al(r0, 16), T), :]
            wt = jnp.concatenate([wqTp[lt] for lt in range(LT)], axis=1)
            pqs[s, 0:T] = _phi(_dot(xa, wt, NT_))

        def nrm(s, T):
            z = zrow[...]
            pq = pqs[s, 0:T]
            sm = pq[:, 0:128] * z[:, 0:128]
            for j in range(1, LT):
                sm = sm + pq[:, 128 * j:128 * (j + 1)] * z[:, 128 * j:128 * (j + 1)]
            sm = sm + pltpu.roll(sm, 64, 1)
            sm = sm + pltpu.roll(sm, 32, 1)
            rr = 1.0 / (sm + 1e-6)
            pqn[s, 0:T] = jnp.concatenate(
                [pq[:, 128 * j:128 * (j + 1)] * rr for j in range(LT)], axis=1).astype(BF16)

        def hs_asm(s, r0, T):
            def hl(j, sh):
                return hbuf[j, pl.ds(r0 + PAD - sh, T), :]
            lane = lax.broadcasted_iota(jnp.int32, (T, 128), 1)
            hsb[s, 0:T] = jnp.concatenate([
                hl(0, 1),
                jnp.where(lane < 32, hl(1, 1), hl(1, -1)),
                jnp.where(lane < 64, hl(2, -1), hl(2, 2)),
                jnp.where(lane < 96, hl(3, 2), hl(3, -2)),
                hl(4, -2)], axis=1).astype(BF16)

        def w2_dot(s, r0, T):
            xa = ax[pl.ds(al(r0, 16), T), :]
            x1 = xa.astype(F32) + _dot(hsb[s, 0:T], w2[...])
            x1s[s, 0:T] = x1
            if ln2out:
                xns[s, 0:T] = x1.astype(BF16)

        def m_dot(s, r0, T):
            a = _dot(pqn[s, 0:T], Mp[...])
            g = gts[pl.ds(al(r0, 16), T), :]
            for j in range(LT):
                sl = slice(128 * j, 128 * (j + 1))
                gas[s, 0:T, sl] = g * a[:, sl] + (1.0 - g) * x1s[s, 0:T, sl]

        def ln2(s, T):
            if not ln2out:
                xns[s, 0:T] = _ln(x1s[s, 0:T]).astype(BF16)

        def w3_dot(s, T):
            xn = xns[s, 0:T]
            if ln2out:
                m, _, rs = _stats(xn.astype(F32))
                rm = rs * m
                gus[s, 0:T, 0:FM] = _gelu(_dot(xn, w3[0:FM, :], NT_) * rs - rm * c3s[:, 0:FM]).astype(BF16)
                ut = _dot(w3[FM:F, :], xn, NT_).T
                gus[s, 0:T, FM:F] = _gelu(ut * rs - rm * c3s[:, FM:F]).astype(BF16)
            else:
                gus[s, 0:T, 0:FM] = _gelu(_dot(xn, w3[0:FM, :], NT_)).astype(BF16)
                ut = _dot(w3[FM:F, :], xn, NT_)
                gus[s, 0:T, FM:F] = _gelu(ut).T.astype(BF16)

        def c3_setup():
            if ln2out:
                cs = _dot(jnp.ones((16, D), BF16), w3[...], NT_)
                c3s[:, 0:F] = cs[0:1, :]

        def ocopy(r0, T, i):
            return pltpu.make_async_copy(ob.at[pl.ds(r0, T), :], out_hbm.at[0, pl.ds(r0, T), :], so.at[i, 0])

        def ocopy_c(r0, T, i, j):
            return pltpu.make_async_copy(ob.at[pl.ds(r0, T), pl.ds(128 * j, 128)],
                                         out_hbm.at[0, pl.ds(r0, T), pl.ds(128 * j, 128)], so.at[i, j])

        def w4_dot(s, r0, T, i, split=False):
            h2 = _dot(gus[s, 0:T, 0:F], w4[...])
            g = gts[pl.ds(al(r0, 16), T), :]
            for j in range(LT):
                sl = slice(128 * j, 128 * (j + 1))
                ob[pl.ds(al(r0, 16), T), sl] = (gas[s, 0:T, sl] + (1.0 - g) * h2[:, sl]).astype(BF16)
                if split:
                    ocopy_c(al(r0, 16), T, i, j).start()
            if not split:
                ocopy(al(r0, 16), T, i).start()

        def kv_dot(j):
            a, b = KV_ROWS[j]
            kvj = _dot(gacc[a:b, :].astype(BF16), wv[:, 128 * j:128 * (j + 1)])
            rh = (lax.broadcasted_iota(jnp.int32, (b - a, 128), 0) + a) // DH
            ch = (lax.broadcasted_iota(jnp.int32, (b - a, 128), 1) + 128 * j) // DH
            return jnp.where(rh == ch, kvj, 0.0).astype(BF16)

        def body_m():
            T = TM[0]

            def fin_a():
                h2 = _dot(gus[0, 0:T, 0:F], w4[...])
                g = gts[0:T, :]
                for j in range(LT):
                    sl = slice(128 * j, 128 * (j + 1))
                    gas[0, 0:T, sl] = (1.0 - g) * (x1s[0, 0:T, sl] + h2[:, sl])

            def fin_b():
                g = gts[0:T, :]
                a = _dot(pqn[0, 0:T], Mp[...])
                for j in range(LT):
                    sl = slice(128 * j, 128 * (j + 1))
                    ob[0:T, sl] = (g * a[:, sl] + gas[0, 0:T, sl]).astype(BF16)
                ocopy(0, T, 0).start()

            def wq_all():
                for lt in range(LT):
                    wq_slice(lt, tmp2, lt)

            if orderM == 0:
                wq_all(); c3_setup()
                kvm = kv_dots()
                hs_asm(0, 0, T); z_setup(); w2_dot(0, 0, T); m_dots(kvm); ln2(0, T); w3_dot(0, T)
                q_dot(0, 0, T); nrm(0, T); fin_a(); fin_b()
            elif orderM == 1:
                wq_all(); c3_setup()
                kvm = [kv_dot(0), kv_dot(1)]
                hs_asm(0, 0, T); w2_dot(0, 0, T)
                kvm += [kv_dot(2), kv_dot(3), kv_dot(4)]
                z_setup(); m_dots(kvm); ln2(0, T); w3_dot(0, T)
                q_dot(0, 0, T); nrm(0, T); fin_a(); fin_b()
            elif orderM == 2:
                wq_all(); c3_setup()
                kvm = [kv_dot(0), kv_dot(1)]
                hs_asm(0, 0, T); w2_dot(0, 0, T)
                kvm += [kv_dot(2), kv_dot(3), kv_dot(4)]
                q_dot(0, 0, T)
                z_setup(); ln2(0, T); w3_dot(0, T)
                m_dots(kvm); nrm(0, T); fin_a(); fin_b()
            elif orderM == 3:
                wq_all(); c3_setup()
                kvm = [kv_dot(0), kv_dot(1)]
                hs_asm(0, 0, T); w2_dot(0, 0, T)
                kvm += [kv_dot(2), kv_dot(3), kv_dot(4)]
                z_setup(); ln2(0, T)
                m_dots(kvm); w3_dot(0, T)
                q_dot(0, 0, T); fin_a(); nrm(0, T); fin_b()

        def body_l(t):
            base = RM + t * BL
            i0 = len(TM) + t * len(TL)
            if len(TL) == 1:
                T = TL[0]
                r0 = al(base, 16)
                q_dot(0, r0, T)
                hs_asm(0, r0, T)
                w2_dot(0, r0, T)
                nrm(0, T)
                m_dot(0, r0, T)
                ln2(0, T)
                w3_dot(0, T)
                w4_dot(0, r0, T, i0)
            else:
                TA, TB = TL
                A, B = al(base, 16), al(base + TA, 16)
                q_dot(0, A, TA)
                hs_asm(0, A, TA)
                w2_dot(0, A, TA)
                q_dot(1, B, TB)
                nrm(0, TA)
                hs_asm(1, B, TB)
                m_dot(0, A, TA)
                w2_dot(1, B, TB)
                ln2(0, TA)
                w3_dot(0, TA)
                nrm(1, TB)
                m_dot(1, B, TB)
                ln2(1, TB)
                w4_dot(0, A, TA, i0)
                w3_dot(1, TB)
                w4_dot(1, B, TB, i0 + 1, split=osplit)

        with scope('pm'):
            for n in late + ['wq']:
                wcopy(n).wait()
            body_m()

        def phase2(t, carry):
            with scope('p2body'):
                body_l(t)
            return carry

        lax.fori_loop(0, N2, phase2, 0)
        with scope('fin'):
            r = 0
            i = 0
            for k, T in enumerate(list(TM) + list(TL) * N2):
                last_sub = osplit and k >= len(TM) and (k - len(TM)) % len(TL) == len(TL) - 1 and len(TL) == 2
                if last_sub:
                    for j in range(LT):
                        ocopy_c(r, T, i, j).wait()
                else:
                    ocopy(r, T, i).wait()
                r += T
                i += 1

    def fn(A_x, A_wqkv, A_wo, B_x, B_w1, B_w2, B_w3, B_w4, gate_w):
        hbm = pl.BlockSpec(memory_space=pltpu.HBM)
        return pl.pallas_call(
            kernel,
            out_shape=jax.ShapeDtypeStruct((1, S, D), BF16),
            in_specs=[hbm] * 8,
            out_specs=hbm,
            scratch_shapes=[
                pltpu.VMEM((S, D), BF16),
                pltpu.VMEM((D, D), BF16), pltpu.VMEM((D, D), BF16), pltpu.VMEM((D, D), BF16),
                pltpu.VMEM((D, D), BF16), pltpu.VMEM((D, D), BF16), pltpu.VMEM((D, D), BF16),
                pltpu.VMEM((F, D), BF16), pltpu.VMEM((F, D), BF16),
                pltpu.VMEM((D,), BF16), pltpu.VMEM((S, D), BF16),
                pltpu.VMEM((D + 16, D), BF16), pltpu.VMEM((LT, D, 128), BF16),
                pltpu.VMEM((LT, D, 128), F32),
                pltpu.VMEM((LT, D, 128), F32),
                pltpu.VMEM((LT, S + 2 * PAD, 128), F32),
                pltpu.VMEM((D, D), F32),
                pltpu.VMEM((D, 128), F32),
                pltpu.VMEM((D, D), BF16),
                pltpu.VMEM((1, D), F32),
                pltpu.VMEM((TF + 16, D), F32),
                pltpu.VMEM((2, TF, 128), F32),
                pltpu.VMEM((1, D), F32),
                pltpu.VMEM((1, 1792), F32),
                pltpu.VMEM((NSL, TMAX, D), F32),
                pltpu.VMEM((NSL, TMAX, D), BF16),
                pltpu.VMEM((NSL, TMAX, D), BF16),
                pltpu.VMEM((NSL, TMAX, D), F32),
                pltpu.VMEM((NSL, TMAX, D), BF16),
                pltpu.VMEM((NSL, TMAX, D), F32),
                pltpu.VMEM((NSL, TMAX, 1792), BF16),
                pltpu.VMEM((S, 128), F32),
                pltpu.SemaphoreType.DMA((NF + NL,)),
                pltpu.SemaphoreType.DMA((14,)),
                pltpu.SemaphoreType.DMA((NOUT, LT)),
            ],
            compiler_params=pltpu.CompilerParams(vmem_limit_bytes=100 * 1024 * 1024, disable_bounds_checks=nobc, disable_semaphore_checks=nosc),
            name='gm',
        )(A_x, A_wqkv, A_wo, B_w1, B_w2, B_w3.T, B_w4, gate_w)
    return fn


_impl = make(nobc=True, osplit=True, nosc=True)


@jax.jit
def pallas_gated_mix__linear_attn_block__mixer_s_mlp__prompt_kernel(A_x, A_wqkv, A_wo, B_x, B_w1, B_w2, B_w3, B_w4, gate_w):
    return _impl(A_x, A_wqkv, A_wo, B_x, B_w1, B_w2, B_w3, B_w4, gate_w)
```

```python
import jax
import jax.numpy as jnp
from jax import lax
from jax.experimental import pallas as pl
from jax.experimental.pallas import tpu as pltpu

S, D, F, H, DH = 2048, 640, 1728, 32, 20
LT = D // 128
FM = (F // 128) * 128
FH = F // 2
PAD = 8
KV_ROWS = ((0, 144), (112, 272), (240, 400), (368, 528), (496, 640))

T0 = 256
KA = 256
N1 = 4
TK = S // N1
HR = 432
NL = N1 - 1
RF = S - NL * HR
T2 = RF - 2 * T0
HA = (HR // 32) * 16
TM = 256
TA, TB = 192, 256
N2 = (S - TM) // (TA + TB)
TMAX = max(TM, TA, TB)
assert T2 > 0 and T2 % 16 == 0 and TM + N2 * (TA + TB) == S

F32 = jnp.float32
BF16 = jnp.bfloat16
NN = (((1,), (0,)), ((), ()))
NT = (((1,), (1,)), ((), ()))

W_A0, W_A1, W_V, W_Q, W_O, W_2, W_3A, W_3B, W_4A, W_4B, W_G, W_K0, W_K1, W_K2 = range(14)
X_0 = 14
O_0 = X_0 + 3 + NL
N_OUT = 1 + N2 * (1 + LT)
N_SEM = O_0 + N_OUT


def _dot(a, b, dims=NN):
    return lax.dot_general(a, b, dims, preferred_element_type=F32)


def _phi(t):
    return jnp.where(t > 0, t + 1.0, jnp.exp(t)) + 1e-6


def _gelu(x):
    c = 0.7978845608028654
    inner = x * (c + (c * 0.044715) * (x * x))
    hx = 0.5 * x
    return hx + hx * jnp.tanh(inner)


def _stats(x):
    m = jnp.mean(x, axis=-1, keepdims=True)
    xc = x - m
    v = jnp.mean(xc * xc, axis=-1, keepdims=True)
    return m, xc, lax.rsqrt(v + 1e-5)


def _al(r, m):
    return r if isinstance(r, int) else pl.multiple_of(r, m)


def _kernel(x_hbm, wqkv_hbm, wo_hbm, w1_hbm, w2_hbm, w3t_hbm, w4_hbm, gw_hbm, out_hbm,
            x, wq, wk, wv, wo, w1, w2, w3t, w4, gw, ob,
            wkt, wqp, tmp_m, tmp_q, hbuf, gacc, zacc, mp, zrow,
            hacc, st0, c1s, pqs, pqn, hsb, x1s, xns, gas, gus, gts, sem):
    def x_copy(r0, n, i):
        return pltpu.make_async_copy(x_hbm.at[0, pl.ds(r0, n), :], x.at[pl.ds(r0, n), :], sem.at[X_0 + i])

    def x_rest(t):
        return x_copy(RF + t * HR, HR, 3 + t)

    def rows_copy(src, dst, r0, n, s):
        return pltpu.make_async_copy(src.at[pl.ds(r0, n), :], dst.at[pl.ds(r0, n), :], sem.at[s])

    def wk_copy(r0, n, s):
        return pltpu.make_async_copy(wqkv_hbm.at[pl.ds(r0, n), pl.ds(D, D)], wk.at[pl.ds(r0, n), :], sem.at[s])

    copies = {
        'a0': lambda: rows_copy(w1_hbm, w1, 0, KA, W_A0),
        'a1': lambda: rows_copy(w1_hbm, w1, KA, D - KA, W_A1),
        'wv': lambda: pltpu.make_async_copy(wqkv_hbm.at[:, pl.ds(2 * D, D)], wv, sem.at[W_V]),
        'wq': lambda: pltpu.make_async_copy(wqkv_hbm.at[:, pl.ds(0, D)], wq, sem.at[W_Q]),
        'wo': lambda: pltpu.make_async_copy(wo_hbm, wo, sem.at[W_O]),
        'w2': lambda: pltpu.make_async_copy(w2_hbm, w2, sem.at[W_2]),
        'w3a': lambda: rows_copy(w3t_hbm, w3t, 0, FH, W_3A),
        'w3b': lambda: rows_copy(w3t_hbm, w3t, FH, FH, W_3B),
        'w4a': lambda: rows_copy(w4_hbm, w4, 0, FH, W_4A),
        'w4b': lambda: rows_copy(w4_hbm, w4, FH, FH, W_4B),
        'gw': lambda: pltpu.make_async_copy(gw_hbm, gw, sem.at[W_G]),
        'k0': lambda: wk_copy(0, 256, W_K0),
        'k1': lambda: wk_copy(256, 256, W_K1),
        'k2': lambda: wk_copy(512, 128, W_K2),
        'x0': lambda: x_copy(0, T0, 0),
        'x1': lambda: x_copy(T0, T0, 1),
        'x2': lambda: x_copy(2 * T0, T2, 2),
        'r0': lambda: x_rest(0),
        'r1': lambda: x_rest(1),
        'r2': lambda: x_rest(2),
    }

    def start(names):
        for n in names.split():
            copies[n]().start()

    def wait(names):
        for n in names.split():
            copies[n]().wait()

    late = ('wv w2', 'wo w3a', 'w3b w4a w4b')

    def out_copy(r0, n, i):
        return pltpu.make_async_copy(ob.at[pl.ds(r0, n), :], out_hbm.at[0, pl.ds(r0, n), :], sem.at[O_0 + i])

    def out_copy_cols(r0, n, i, j):
        return pltpu.make_async_copy(ob.at[pl.ds(r0, n), pl.ds(128 * j, 128)],
                                     out_hbm.at[0, pl.ds(r0, n), pl.ds(128 * j, 128)], sem.at[O_0 + i + j])

    def tile(j):
        return slice(128 * j, 128 * (j + 1))

    def h_dot(r0, n):
        xa = x[pl.ds(_al(r0, 16), n), :]
        y = _dot(xa, w1[...])
        m, _, rs = _stats(xa.astype(F32))
        h = _gelu(y * rs - (rs * m) * c1s[...])
        for j in range(LT):
            hbuf[j, pl.ds(_al(r0 + PAD, 8), n), :] = h[:, tile(j)]

    def k_dot(r0, n):
        kk = _dot(wkt[...], x[pl.ds(_al(r0, 16), n), :], NT)
        pk = _phi(kk[0:D, :])
        g = 0.5 * jnp.tanh(0.5 * kk[D:D + 1, :]) + 0.5
        gts[pl.ds(_al(r0, 128), n), :] = jnp.broadcast_to(g, (128, n)).T
        zs = pk[:, 0:128]
        for j in range(1, n // 128):
            zs = zs + pk[:, tile(j)]
        return pk.astype(BF16), zs

    start('x0 gw a0')
    for j in range(LT):
        hbuf[j, 0:PAD, :] = jnp.zeros((PAD, 128), F32)
        hbuf[j, PAD + S:PAD + S + PAD, :] = jnp.zeros((PAD, 128), F32)
    ones = jnp.ones((16, D), BF16)
    wait('x0')
    start('a1 x1')
    wait('gw')
    m0, _, rs0 = _stats(x[0:T0, :].astype(F32))
    st0[0] = jnp.broadcast_to(rs0, (T0, 128))
    st0[1] = jnp.broadcast_to(rs0 * m0, (T0, 128))
    wait('a0')
    start('k0 x2 k1 k2')
    hacc[...] = _dot(jnp.concatenate([ones[:, 0:KA], x[0:T0, 0:KA]], axis=0), w1[0:KA, :])
    wait('a1')
    start('r0 wq')
    y0 = hacc[...] + _dot(jnp.concatenate([ones[:, KA:D], x[0:T0, KA:D]], axis=0), w1[KA:D, :])
    c1 = y0[0:1, :]
    c1s[...] = c1
    for j in range(LT):
        hbuf[j, PAD:PAD + T0, :] = _gelu(y0[16:16 + T0, tile(j)] * st0[0] - st0[1] * c1[:, tile(j)])
    wait('x1')
    start('r1 r2')
    h_dot(T0, T0)
    wait('k0 x2 k1 k2')
    start(late[0])
    for a, b in ((0, 256), (256, 512), (512, 640)):
        wkt[0:D, a:b] = wk[a:b, :].T
    row = lax.broadcasted_iota(jnp.int32, (16, D), 0)
    wkt[D:D + 16, :] = jnp.where(
        row == 0, jnp.broadcast_to(gw[...].astype(F32).reshape(1, D), (16, D)), 0.0).astype(BF16)
    h_dot(2 * T0, T2)
    th = TK // 2
    pka, zsa = k_dot(0, th)
    pkb, zsb = k_dot(th, th)
    zacc[...] = zsa + zsb
    ga0 = _dot(pka, x[0:th, :])
    gacc[...] = ga0 + _dot(pkb, x[th:TK, :])

    def phase1(t, carry):
        x_rest(t).wait()
        r0 = _al((t + 1) * TK, 128)
        h_dot(RF + t * HR, HA)
        pk, zs = k_dot(r0, TK)
        h_dot(RF + t * HR + HA, HR - HA)
        zacc[...] += zs
        gacc[...] += _dot(pk, x[pl.ds(r0, TK), :])
        for i in range(1, NL):
            @pl.when(t == i - 1)
            def _(i=i):
                start(late[i])
        return carry

    lax.fori_loop(0, NL, phase1, 0)

    def wq_permute():
        for lt in range(LT):
            tmp_q[lt] = wq[tile(lt), :].T.astype(F32)
            for j in range(LT):
                for c in range(4):
                    wqp[lt, pl.ds(128 * j + 32 * c, 32), :] = (
                        tmp_q[lt, pl.ds(4 * j + c, 32, stride=DH), :].astype(BF16))

    def kv_dot(j):
        a, b = KV_ROWS[j]
        kv = _dot(gacc[a:b, :].astype(BF16), wv[:, tile(j)])
        rh = (lax.broadcasted_iota(jnp.int32, (b - a, 128), 0) + a) // DH
        ch = (lax.broadcasted_iota(jnp.int32, (b - a, 128), 1) + 128 * j) // DH
        return jnp.where(rh == ch, kv, 0.0).astype(BF16)

    def m_dots(kvs):
        carry = None
        for j in range(LT):
            a, b = KV_ROWS[j]
            part = _dot(kvs[j], wo[tile(j), :])
            lo = 0
            if carry is not None:
                head = part[0:32, :] + carry
                for lt in range(LT):
                    tmp_m[lt, a:a + 32, :] = head[:, tile(lt)]
                lo = 32
            hi = (b - a) - (32 if j + 1 < LT else 0)
            for lt in range(LT):
                tmp_m[lt, a + lo:a + hi, :] = part[lo:hi, tile(lt)]
            carry = part[hi:b - a, :] if j + 1 < LT else None
        for j in range(LT):
            for c in range(4):
                for lt in range(LT):
                    mp[pl.ds(128 * j + 32 * c, 32), tile(lt)] = (
                        tmp_m[lt, pl.ds(4 * j + c, 32, stride=DH), :].astype(BF16))

    def z_setup():
        for j in range(LT):
            zp = jnp.concatenate([zacc[pl.ds(4 * j + c, 32, stride=DH), :] for c in range(4)], axis=0)
            zrow[:, tile(j)] = jnp.sum(zp.T, axis=0, keepdims=True)

    def q_dot(s, r0, n):
        wt = jnp.concatenate([wqp[lt] for lt in range(LT)], axis=1)
        pqs[s, 0:n] = _phi(_dot(x[pl.ds(_al(r0, 16), n), :], wt, NT))

    def normalize(s, n):
        z = zrow[...]
        pq = pqs[s, 0:n]
        den = pq[:, tile(0)] * z[:, tile(0)]
        for j in range(1, LT):
            den = den + pq[:, tile(j)] * z[:, tile(j)]
        den = den + pltpu.roll(den, 64, 1)
        den = den + pltpu.roll(den, 32, 1)
        inv = 1.0 / (den + 1e-6)
        pqn[s, 0:n] = jnp.concatenate([pq[:, tile(j)] * inv for j in range(LT)], axis=1).astype(BF16)

    def shift(s, r0, n):
        def hl(j, sh):
            return hbuf[j, pl.ds(r0 + PAD - sh, n), :]
        lane = lax.broadcasted_iota(jnp.int32, (n, 128), 1)
        hsb[s, 0:n] = jnp.concatenate([
            hl(0, 1),
            jnp.where(lane < 32, hl(1, 1), hl(1, -1)),
            jnp.where(lane < 64, hl(2, -1), hl(2, 2)),
            jnp.where(lane < 96, hl(3, 2), hl(3, -2)),
            hl(4, -2)], axis=1).astype(BF16)

    def w2_dot(s, r0, n):
        x1s[s, 0:n] = x[pl.ds(_al(r0, 16), n), :].astype(F32) + _dot(hsb[s, 0:n], w2[...])

    def m_dot(s, r0, n):
        a = _dot(pqn[s, 0:n], mp[...])
        g = gts[pl.ds(_al(r0, 16), n), :]
        for j in range(LT):
            gas[s, 0:n, tile(j)] = g * a[:, tile(j)] + (1.0 - g) * x1s[s, 0:n, tile(j)]

    def ln2(s, n):
        _, xc, rs = _stats(x1s[s, 0:n])
        xns[s, 0:n] = (xc * rs).astype(BF16)

    def w3_dot(s, n):
        xn = xns[s, 0:n]
        gus[s, 0:n, 0:FM] = _gelu(_dot(xn, w3t[0:FM, :], NT)).astype(BF16)
        ut = _dot(w3t[FM:F, :], xn, NT)
        gus[s, 0:n, FM:F] = _gelu(ut).T.astype(BF16)

    def w4_dot(s, r0, n, i, by_cols):
        h2 = _dot(gus[s, 0:n, 0:F], w4[...])
        r0 = _al(r0, 16)
        g = gts[pl.ds(r0, n), :]
        for j in range(LT):
            ob[pl.ds(r0, n), tile(j)] = (gas[s, 0:n, tile(j)] + (1.0 - g) * h2[:, tile(j)]).astype(BF16)
            if by_cols:
                out_copy_cols(r0, n, i, j).start()
        if not by_cols:
            out_copy(r0, n, i).start()

    wait('wv w2 wo w3a w3b w4a w4b wq')
    wq_permute()
    kvs = [kv_dot(0), kv_dot(1)]
    shift(0, 0, TM)
    w2_dot(0, 0, TM)
    kvs += [kv_dot(2), kv_dot(3), kv_dot(4)]
    z_setup()
    m_dots(kvs)
    ln2(0, TM)
    w3_dot(0, TM)
    q_dot(0, 0, TM)
    normalize(0, TM)
    h2_0 = _dot(gus[0, 0:TM, 0:F], w4[...])
    g_0 = gts[0:TM, :]
    for j in range(LT):
        gas[0, 0:TM, tile(j)] = (1.0 - g_0) * (x1s[0, 0:TM, tile(j)] + h2_0[:, tile(j)])
    a_0 = _dot(pqn[0, 0:TM], mp[...])
    for j in range(LT):
        ob[0:TM, tile(j)] = (g_0 * a_0[:, tile(j)] + gas[0, 0:TM, tile(j)]).astype(BF16)
    out_copy(0, TM, 0).start()

    def phase2(t, carry):
        ra = _al(TM + t * (TA + TB), 16)
        rb = _al(ra + TA, 16)
        i0 = 1 + t * (1 + LT)
        q_dot(0, ra, TA)
        shift(0, ra, TA)
        w2_dot(0, ra, TA)
        q_dot(1, rb, TB)
        normalize(0, TA)
        shift(1, rb, TB)
        m_dot(0, ra, TA)
        w2_dot(1, rb, TB)
        ln2(0, TA)
        w3_dot(0, TA)
        normalize(1, TB)
        m_dot(1, rb, TB)
        ln2(1, TB)
        w4_dot(0, ra, TA, i0, False)
        w3_dot(1, TB)
        w4_dot(1, rb, TB, i0 + 1, True)
        return carry

    lax.fori_loop(0, N2, phase2, 0)

    out_copy(0, TM, 0).wait()
    for t in range(N2):
        ra = TM + t * (TA + TB)
        i0 = 1 + t * (1 + LT)
        out_copy(ra, TA, i0).wait()
        for j in range(LT):
            out_copy_cols(ra + TA, TB, i0 + 1, j).wait()


@jax.jit
def pallas_gated_mix__linear_attn_block__mixer_s_mlp__prompt_kernel(
        A_x, A_wqkv, A_wo, B_x, B_w1, B_w2, B_w3, B_w4, gate_w):
    del B_x
    hbm = pl.BlockSpec(memory_space=pltpu.HBM)
    vmem = pltpu.VMEM
    return pl.pallas_call(
        _kernel,
        out_shape=jax.ShapeDtypeStruct((1, S, D), BF16),
        in_specs=[hbm] * 8,
        out_specs=hbm,
        scratch_shapes=[
            vmem((S, D), BF16),
            vmem((D, D), BF16), vmem((D, D), BF16), vmem((D, D), BF16),
            vmem((D, D), BF16), vmem((D, D), BF16), vmem((D, D), BF16),
            vmem((F, D), BF16), vmem((F, D), BF16),
            vmem((D,), BF16), vmem((S, D), BF16),
            vmem((D + 16, D), BF16),
            vmem((LT, D, 128), BF16),
            vmem((LT, D, 128), F32),
            vmem((LT, D, 128), F32),
            vmem((LT, S + 2 * PAD, 128), F32),
            vmem((D, D), F32),
            vmem((D, 128), F32),
            vmem((D, D), BF16),
            vmem((1, D), F32),
            vmem((T0 + 16, D), F32),
            vmem((2, T0, 128), F32),
            vmem((1, D), F32),
            vmem((2, TMAX, D), F32),
            vmem((2, TMAX, D), BF16),
            vmem((2, TMAX, D), BF16),
            vmem((2, TMAX, D), F32),
            vmem((2, TMAX, D), BF16),
            vmem((2, TMAX, D), F32),
            vmem((2, TMAX, F), BF16),
            vmem((S, 128), F32),
            pltpu.SemaphoreType.DMA((N_SEM,)),
        ],
        compiler_params=pltpu.CompilerParams(
            vmem_limit_bytes=100 * 1024 * 1024,
            disable_bounds_checks=True,
            disable_semaphore_checks=True,
        ),
        name='gm',
    )(A_x, A_wqkv, A_wo, B_w1, B_w2, B_w3.T, B_w4, gate_w)
```

```python
import jax
import jax.numpy as jnp
from jax import lax
from jax.experimental import pallas as pl
from jax.experimental.pallas import tpu as pltpu

S, D, F, H, DH = 2048, 640, 1728, 32, 20
LT = D // 128
FM = (F // 128) * 128
FH = F // 2
PAD = 8
KV_ROWS = ((0, 144), (112, 272), (240, 400), (368, 528), (496, 640))

T0 = 256
KA = 256
N1 = 4
TK = S // N1
HR = 432
NL = N1 - 1
RF = S - NL * HR
T2 = RF - 2 * T0
HA = (HR // 32) * 16
TM = 256
TA, TB = 192, 256
N2 = (S - TM) // (TA + TB)
TMAX = max(TM, TA, TB)
assert T2 > 0 and T2 % 16 == 0 and TM + N2 * (TA + TB) == S

F32 = jnp.float32
BF16 = jnp.bfloat16
NN = (((1,), (0,)), ((), ()))
NT = (((1,), (1,)), ((), ()))

W_A0, W_A1, W_V, W_Q, W_O, W_2, W_3A, W_3B, W_4A, W_4B, W_G, W_K0, W_K1, W_K2 = range(14)
X_0 = 14
O_0 = X_0 + 3 + NL
N_OUT = 1 + N2 * (1 + LT)
N_SEM = O_0 + N_OUT


def _dot(a, b, dims=NN):
    return lax.dot_general(a, b, dims, preferred_element_type=F32)


def _phi(t):
    return jnp.where(t > 0, t + 1.0, jnp.exp(t)) + 1e-6


def _gelu(x):
    c = 0.7978845608028654
    inner = x * (c + (c * 0.044715) * (x * x))
    hx = 0.5 * x
    return hx + hx * jnp.tanh(inner)


def _stats(x):
    m = jnp.mean(x, axis=-1, keepdims=True)
    xc = x - m
    v = jnp.mean(xc * xc, axis=-1, keepdims=True)
    return m, xc, lax.rsqrt(v + 1e-5)


def _al(r, m):
    return r if isinstance(r, int) else pl.multiple_of(r, m)


def _kernel(x_hbm, wqkv_hbm, wo_hbm, w1_hbm, w2_hbm, w3t_hbm, w4_hbm, gw_hbm, out_hbm,
            x, wq, wk, wv, wo, w1, w2, w3t, w4, gw, ob,
            wkt, wqp, tmp_m, tmp_q, hbuf, gacc, zacc, mp, zrow,
            hacc, st0, c1s, pqs, pqn, hsb, x1s, xns, gas, gus, gts, sem):
    def x_copy(r0, n, i):
        return pltpu.make_async_copy(x_hbm.at[0, pl.ds(r0, n), :], x.at[pl.ds(r0, n), :], sem.at[X_0 + i])

    def x_rest(t):
        return x_copy(RF + t * HR, HR, 3 + t)

    def rows_copy(src, dst, r0, n, s):
        return pltpu.make_async_copy(src.at[pl.ds(r0, n), :], dst.at[pl.ds(r0, n), :], sem.at[s])

    def wk_copy(r0, n, s):
        return pltpu.make_async_copy(wqkv_hbm.at[pl.ds(r0, n), pl.ds(D, D)], wk.at[pl.ds(r0, n), :], sem.at[s])

    copies = {
        'a0': lambda: rows_copy(w1_hbm, w1, 0, KA, W_A0),
        'a1': lambda: rows_copy(w1_hbm, w1, KA, D - KA, W_A1),
        'wv': lambda: pltpu.make_async_copy(wqkv_hbm.at[:, pl.ds(2 * D, D)], wv, sem.at[W_V]),
        'wq': lambda: pltpu.make_async_copy(wqkv_hbm.at[:, pl.ds(0, D)], wq, sem.at[W_Q]),
        'wo': lambda: pltpu.make_async_copy(wo_hbm, wo, sem.at[W_O]),
        'w2': lambda: pltpu.make_async_copy(w2_hbm, w2, sem.at[W_2]),
        'w3a': lambda: rows_copy(w3t_hbm, w3t, 0, FH, W_3A),
        'w3b': lambda: rows_copy(w3t_hbm, w3t, FH, FH, W_3B),
        'w4a': lambda: rows_copy(w4_hbm, w4, 0, FH, W_4A),
        'w4b': lambda: rows_copy(w4_hbm, w4, FH, FH, W_4B),
        'gw': lambda: pltpu.make_async_copy(gw_hbm, gw, sem.at[W_G]),
        'k0': lambda: wk_copy(0, 256, W_K0),
        'k1': lambda: wk_copy(256, 256, W_K1),
        'k2': lambda: wk_copy(512, 128, W_K2),
        'x0': lambda: x_copy(0, T0, 0),
        'x1': lambda: x_copy(T0, T0, 1),
        'x2': lambda: x_copy(2 * T0, T2, 2),
        'r0': lambda: x_rest(0),
        'r1': lambda: x_rest(1),
        'r2': lambda: x_rest(2),
    }

    def start(names):
        for n in names.split():
            copies[n]().start()

    def wait(names):
        for n in names.split():
            copies[n]().wait()

    late = ('wv w2', 'wo w3a', 'w3b w4a w4b')

    def out_copy(r0, n, i):
        return pltpu.make_async_copy(ob.at[pl.ds(r0, n), :], out_hbm.at[0, pl.ds(r0, n), :], sem.at[O_0 + i])

    def out_copy_cols(r0, n, i, j):
        return pltpu.make_async_copy(ob.at[pl.ds(r0, n), pl.ds(128 * j, 128)],
                                     out_hbm.at[0, pl.ds(r0, n), pl.ds(128 * j, 128)], sem.at[O_0 + i + j])

    def tile(j):
        return slice(128 * j, 128 * (j + 1))

    def h_dot(r0, n):
        xa = x[pl.ds(_al(r0, 16), n), :]
        y = _dot(xa, w1[...])
        m, _, rs = _stats(xa.astype(F32))
        h = _gelu(y * rs - (rs * m) * c1s[...])
        for j in range(LT):
            hbuf[j, pl.ds(_al(r0 + PAD, 8), n), :] = h[:, tile(j)]

    def k_dot(r0, n):
        kk = _dot(wkt[...], x[pl.ds(_al(r0, 16), n), :], NT)
        pk = _phi(kk[0:D, :])
        g = 0.5 * jnp.tanh(0.5 * kk[D:D + 1, :]) + 0.5
        gts[pl.ds(_al(r0, 128), n), :] = jnp.broadcast_to(g, (128, n)).T
        zs = pk[:, 0:128]
        for j in range(1, n // 128):
            zs = zs + pk[:, tile(j)]
        return pk.astype(BF16), zs

    start('x0 gw a0')
    for j in range(LT):
        hbuf[j, 0:PAD, :] = jnp.zeros((PAD, 128), F32)
        hbuf[j, PAD + S:PAD + S + PAD, :] = jnp.zeros((PAD, 128), F32)
    ones = jnp.ones((16, D), BF16)
    wait('x0')
    start('a1 x1')
    wait('gw')
    m0, _, rs0 = _stats(x[0:T0, :].astype(F32))
    st0[0] = jnp.broadcast_to(rs0, (T0, 128))
    st0[1] = jnp.broadcast_to(rs0 * m0, (T0, 128))
    wait('a0')
    start('k0 x2 k1 k2')
    hacc[...] = _dot(jnp.concatenate([ones[:, 0:KA], x[0:T0, 0:KA]], axis=0), w1[0:KA, :])
    wait('a1')
    start('r0 wq')
    y0 = hacc[...] + _dot(jnp.concatenate([ones[:, KA:D], x[0:T0, KA:D]], axis=0), w1[KA:D, :])
    c1 = y0[0:1, :]
    c1s[...] = c1
    for j in range(LT):
        hbuf[j, PAD:PAD + T0, :] = _gelu(y0[16:16 + T0, tile(j)] * st0[0] - st0[1] * c1[:, tile(j)])
    wait('x1')
    start('r1 r2')
    h_dot(T0, T0)
    wait('k0 x2 k1 k2')
    start(late[0])
    for a, b in ((0, 256), (256, 512), (512, 640)):
        wkt[0:D, a:b] = wk[a:b, :].T
    row = lax.broadcasted_iota(jnp.int32, (16, D), 0)
    wkt[D:D + 16, :] = jnp.where(
        row == 0, jnp.broadcast_to(gw[...].astype(F32).reshape(1, D), (16, D)), 0.0).astype(BF16)
    h_dot(2 * T0, T2)
    th = TK // 2
    pka, zsa = k_dot(0, th)
    pkb, zsb = k_dot(th, th)
    zacc[...] = zsa + zsb
    ga0 = _dot(pka, x[0:th, :])
    gacc[...] = ga0 + _dot(pkb, x[th:TK, :])

    def phase1(t, carry):
        x_rest(t).wait()
        r0 = _al((t + 1) * TK, 128)
        h_dot(RF + t * HR, HA)
        pk, zs = k_dot(r0, TK)
        h_dot(RF + t * HR + HA, HR - HA)
        zacc[...] += zs
        gacc[...] += _dot(pk, x[pl.ds(r0, TK), :])
        for i in range(1, NL):
            @pl.when(t == i - 1)
            def _(i=i):
                start(late[i])
        return carry

    lax.fori_loop(0, NL, phase1, 0)

    def wq_permute():
        for lt in range(LT):
            tmp_q[lt] = wq[tile(lt), :].T.astype(F32)
            for j in range(LT):
                for c in range(4):
                    wqp[lt, pl.ds(128 * j + 32 * c, 32), :] = (
                        tmp_q[lt, pl.ds(4 * j + c, 32, stride=DH), :].astype(BF16))

    def kv_dot(j):
        a, b = KV_ROWS[j]
        kv = _dot(gacc[a:b, :].astype(BF16), wv[:, tile(j)])
        rh = (lax.broadcasted_iota(jnp.int32, (b - a, 128), 0) + a) // DH
        ch = (lax.broadcasted_iota(jnp.int32, (b - a, 128), 1) + 128 * j) // DH
        return jnp.where(rh == ch, kv, 0.0).astype(BF16)

    def m_dots(kvs):
        carry = None
        for j in range(LT):
            a, b = KV_ROWS[j]
            part = _dot(kvs[j], wo[tile(j), :])
            lo = 0
            if carry is not None:
                head = part[0:32, :] + carry
                for lt in range(LT):
                    tmp_m[lt, a:a + 32, :] = head[:, tile(lt)]
                lo = 32
            hi = (b - a) - (32 if j + 1 < LT else 0)
            for lt in range(LT):
                tmp_m[lt, a + lo:a + hi, :] = part[lo:hi, tile(lt)]
            carry = part[hi:b - a, :] if j + 1 < LT else None
        for j in range(LT):
            for c in range(4):
                for lt in range(LT):
                    mp[pl.ds(128 * j + 32 * c, 32), tile(lt)] = (
                        tmp_m[lt, pl.ds(4 * j + c, 32, stride=DH), :].astype(BF16))

    def z_setup():
        for j in range(LT):
            zp = jnp.concatenate([zacc[pl.ds(4 * j + c, 32, stride=DH), :] for c in range(4)], axis=0)
            zrow[:, tile(j)] = jnp.sum(zp.T, axis=0, keepdims=True)

    def q_dot(s, r0, n):
        wt = jnp.concatenate([wqp[lt] for lt in range(LT)], axis=1)
        pqs[s, 0:n] = _phi(_dot(x[pl.ds(_al(r0, 16), n), :], wt, NT))

    def normalize(s, n):
        z = zrow[...]
        pq = pqs[s, 0:n]
        den = pq[:, tile(0)] * z[:, tile(0)]
        for j in range(1, LT):
            den = den + pq[:, tile(j)] * z[:, tile(j)]
        den = den + pltpu.roll(den, 64, 1)
        den = den + pltpu.roll(den, 32, 1)
        inv = 1.0 / (den + 1e-6)
        pqn[s, 0:n] = jnp.concatenate([pq[:, tile(j)] * inv for j in range(LT)], axis=1).astype(BF16)

    def shift(s, r0, n):
        def hl(j, sh):
            return hbuf[j, pl.ds(r0 + PAD - sh, n), :]
        lane = lax.broadcasted_iota(jnp.int32, (n, 128), 1)
        hsb[s, 0:n] = jnp.concatenate([
            hl(0, 1),
            jnp.where(lane < 32, hl(1, 1), hl(1, -1)),
            jnp.where(lane < 64, hl(2, -1), hl(2, 2)),
            jnp.where(lane < 96, hl(3, 2), hl(3, -2)),
            hl(4, -2)], axis=1).astype(BF16)

    def w2_dot(s, r0, n):
        x1s[s, 0:n] = x[pl.ds(_al(r0, 16), n), :].astype(F32) + _dot(hsb[s, 0:n], w2[...])

    def m_dot(s, r0, n):
        a = _dot(pqn[s, 0:n], mp[...])
        g = gts[pl.ds(_al(r0, 16), n), :]
        for j in range(LT):
            gas[s, 0:n, tile(j)] = g * a[:, tile(j)] + (1.0 - g) * x1s[s, 0:n, tile(j)]

    def ln2(s, n):
        _, xc, rs = _stats(x1s[s, 0:n])
        xns[s, 0:n] = (xc * rs).astype(BF16)

    def w3_dot(s, n):
        xn = xns[s, 0:n]
        gus[s, 0:n, 0:FM] = _gelu(_dot(xn, w3t[0:FM, :], NT)).astype(BF16)
        ut = _dot(w3t[FM:F, :], xn, NT)
        gus[s, 0:n, FM:F] = _gelu(ut).T.astype(BF16)

    def w4_dot(s, r0, n, i, by_cols):
        h2 = _dot(gus[s, 0:n, 0:F], w4[...])
        r0 = _al(r0, 16)
        g = gts[pl.ds(r0, n), :]
        for j in range(LT):
            ob[pl.ds(r0, n), tile(j)] = (gas[s, 0:n, tile(j)] + (1.0 - g) * h2[:, tile(j)]).astype(BF16)
            if by_cols:
                out_copy_cols(r0, n, i, j).start()
        if not by_cols:
            out_copy(r0, n, i).start()

    wait('wv w2 wo w3a w3b w4a w4b wq')
    wq_permute()
    kvs = [kv_dot(0), kv_dot(1)]
    shift(0, 0, TM)
    w2_dot(0, 0, TM)
    kvs += [kv_dot(2), kv_dot(3), kv_dot(4)]
    z_setup()
    m_dots(kvs)
    ln2(0, TM)
    w3_dot(0, TM)
    q_dot(0, 0, TM)
    normalize(0, TM)
    h2_0 = _dot(gus[0, 0:TM, 0:F], w4[...])
    g_0 = gts[0:TM, :]
    for j in range(LT):
        gas[0, 0:TM, tile(j)] = (1.0 - g_0) * (x1s[0, 0:TM, tile(j)] + h2_0[:, tile(j)])
    a_0 = _dot(pqn[0, 0:TM], mp[...])
    for j in range(LT):
        ob[0:TM, tile(j)] = (g_0 * a_0[:, tile(j)] + gas[0, 0:TM, tile(j)]).astype(BF16)
    out_copy(0, TM, 0).start()

    def phase2(t, carry):
        ra = _al(TM + t * (TA + TB), 16)
        rb = _al(ra + TA, 16)
        i0 = 1 + t * (1 + LT)
        q_dot(0, ra, TA)
        shift(0, ra, TA)
        w2_dot(0, ra, TA)
        q_dot(1, rb, TB)
        normalize(0, TA)
        shift(1, rb, TB)
        m_dot(0, ra, TA)
        w2_dot(1, rb, TB)
        ln2(0, TA)
        w3_dot(0, TA)
        normalize(1, TB)
        m_dot(1, rb, TB)
        ln2(1, TB)
        w4_dot(0, ra, TA, i0, False)
        w3_dot(1, TB)
        w4_dot(1, rb, TB, i0 + 1, True)
        return carry

    lax.fori_loop(0, N2, phase2, 0)

    out_copy(0, TM, 0).wait()
    for t in range(N2):
        ra = TM + t * (TA + TB)
        i0 = 1 + t * (1 + LT)
        out_copy(ra, TA, i0).wait()
        for j in range(LT):
            out_copy_cols(ra + TA, TB, i0 + 1, j).wait()


def _compiler_params():
    vmem = dict(vmem_limit_bytes=100 * 1024 * 1024)
    try:
        return pltpu.CompilerParams(disable_bounds_checks=True, disable_semaphore_checks=True, **vmem)
    except TypeError:
        return pltpu.CompilerParams(**vmem)


@jax.jit
def pallas_gated_mix__linear_attn_block__mixer_s_mlp__prompt_kernel(
        A_x, A_wqkv, A_wo, B_x, B_w1, B_w2, B_w3, B_w4, gate_w):
    del B_x
    hbm = pl.BlockSpec(memory_space=pltpu.MemorySpace.HBM)
    vmem = pltpu.VMEM
    return pl.pallas_call(
        _kernel,
        out_shape=jax.ShapeDtypeStruct((1, S, D), BF16),
        in_specs=[hbm] * 8,
        out_specs=hbm,
        scratch_shapes=[
            vmem((S, D), BF16),
            vmem((D, D), BF16), vmem((D, D), BF16), vmem((D, D), BF16),
            vmem((D, D), BF16), vmem((D, D), BF16), vmem((D, D), BF16),
            vmem((F, D), BF16), vmem((F, D), BF16),
            vmem((D,), BF16), vmem((S, D), BF16),
            vmem((D + 16, D), BF16),
            vmem((LT, D, 128), BF16),
            vmem((LT, D, 128), F32),
            vmem((LT, D, 128), F32),
            vmem((LT, S + 2 * PAD, 128), F32),
            vmem((D, D), F32),
            vmem((D, 128), F32),
            vmem((D, D), BF16),
            vmem((1, D), F32),
            vmem((T0 + 16, D), F32),
            vmem((2, T0, 128), F32),
            vmem((1, D), F32),
            vmem((2, TMAX, D), F32),
            vmem((2, TMAX, D), BF16),
            vmem((2, TMAX, D), BF16),
            vmem((2, TMAX, D), F32),
            vmem((2, TMAX, D), BF16),
            vmem((2, TMAX, D), F32),
            vmem((2, TMAX, F), BF16),
            vmem((S, 128), F32),
            pltpu.SemaphoreType.DMA((N_SEM,)),
        ],
        compiler_params=_compiler_params(),
        name='gm',
    )(A_x, A_wqkv, A_wo, B_w1, B_w2, B_w3.T, B_w4, gate_w)
```

```python
import jax
import jax.numpy as jnp
from jax import lax
from jax.experimental import pallas as pl
from jax.experimental.pallas import tpu as pltpu

S, D, F, H, DH = 2048, 640, 1728, 32, 20
LT = D // 128
FM = (F // 128) * 128
FH = F // 2
PAD = 8
KV_ROWS = ((0, 144), (112, 272), (240, 400), (368, 528), (496, 640))

T0 = 256
T1 = 352
KA = 256
N1 = 4
TK = S // N1
HR = 432
NL = N1 - 1
RF = S - NL * HR
T2 = RF - T0 - T1
HA = (HR // 32) * 16
TM = 256
TA, TB = 192, 256
N2 = (S - TM) // (TA + TB)
TMAX = max(TM, TA, TB)
assert T2 > 0 and T2 % 16 == 0 and T1 % 32 == 0 and TM + N2 * (TA + TB) == S

F32 = jnp.float32
BF16 = jnp.bfloat16
NN = (((1,), (0,)), ((), ()))
NT = (((1,), (1,)), ((), ()))

W_A0, W_A1, W_V, W_Q, W_O, W_2, W_3A, W_3B, W_4A, W_4B, W_G, W_K = range(12)
X_0 = 12
O_0 = X_0 + 3 + NL
N_OUT = 1 + N2 * (1 + LT)
N_SEM = O_0 + N_OUT


def _dot(a, b, dims=NN):
    return lax.dot_general(a, b, dims, preferred_element_type=F32)


def _phi(t):
    return jnp.where(t > 0, t + 1.0, jnp.exp(t)) + 1e-6


def _gelu(x):
    c = 0.7978845608028654
    inner = x * (c + (c * 0.044715) * (x * x))
    hx = 0.5 * x
    return hx + hx * jnp.tanh(inner)


def _stats(x):
    m = jnp.mean(x, axis=-1, keepdims=True)
    xc = x - m
    v = jnp.mean(xc * xc, axis=-1, keepdims=True)
    return m, xc, lax.rsqrt(v + 1e-5)


def _al(r, m):
    return r if isinstance(r, int) else pl.multiple_of(r, m)


def _kernel(x_hbm, wqkv_hbm, wo_hbm, w1_hbm, w2_hbm, w3t_hbm, w4_hbm, gw_hbm, out_hbm,
            x, wq, wk, wv, wo, w1, w2, w3t, w4, gw, ob,
            wkt, wqp, tmp_m, tmp_q, hbuf, gacc, zacc, mp, zrow,
            hacc, st0, c1s, pqs, pqn, hsb, x1s, xns, gas, gus, gts, sem):
    def x_copy(r0, n, i):
        return pltpu.make_async_copy(x_hbm.at[0, pl.ds(r0, n), :], x.at[pl.ds(r0, n), :], sem.at[X_0 + i])

    def x_rest(t):
        return x_copy(RF + t * HR, HR, 3 + t)

    def rows_copy(src, dst, r0, n, s):
        return pltpu.make_async_copy(src.at[pl.ds(r0, n), :], dst.at[pl.ds(r0, n), :], sem.at[s])

    copies = {
        'a0': lambda: rows_copy(w1_hbm, w1, 0, KA, W_A0),
        'a1': lambda: rows_copy(w1_hbm, w1, KA, D - KA, W_A1),
        'wv': lambda: pltpu.make_async_copy(wqkv_hbm.at[:, pl.ds(2 * D, D)], wv, sem.at[W_V]),
        'wq': lambda: pltpu.make_async_copy(wqkv_hbm.at[:, pl.ds(0, D)], wq, sem.at[W_Q]),
        'wo': lambda: pltpu.make_async_copy(wo_hbm, wo, sem.at[W_O]),
        'w2': lambda: pltpu.make_async_copy(w2_hbm, w2, sem.at[W_2]),
        'w3a': lambda: rows_copy(w3t_hbm, w3t, 0, FH, W_3A),
        'w3b': lambda: rows_copy(w3t_hbm, w3t, FH, FH, W_3B),
        'w4a': lambda: rows_copy(w4_hbm, w4, 0, FH, W_4A),
        'w4b': lambda: rows_copy(w4_hbm, w4, FH, FH, W_4B),
        'gw': lambda: pltpu.make_async_copy(gw_hbm, gw, sem.at[W_G]),
        'wk': lambda: pltpu.make_async_copy(wqkv_hbm.at[:, pl.ds(D, D)], wk, sem.at[W_K]),
        'x0': lambda: x_copy(0, T0, 0),
        'x1': lambda: x_copy(T0, T1, 1),
        'x2': lambda: x_copy(T0 + T1, T2, 2),
        'r0': lambda: x_rest(0),
        'r1': lambda: x_rest(1),
        'r2': lambda: x_rest(2),
    }

    def start(names):
        for n in names.split():
            copies[n]().start()

    def wait(names):
        for n in names.split():
            copies[n]().wait()

    late = ('wv w2', 'wo w3a', 'w3b w4a w4b')

    def out_copy(r0, n, i):
        return pltpu.make_async_copy(ob.at[pl.ds(r0, n), :], out_hbm.at[0, pl.ds(r0, n), :], sem.at[O_0 + i])

    def out_copy_cols(r0, n, i, j):
        return pltpu.make_async_copy(ob.at[pl.ds(r0, n), pl.ds(128 * j, 128)],
                                     out_hbm.at[0, pl.ds(r0, n), pl.ds(128 * j, 128)], sem.at[O_0 + i + j])

    def tile(j):
        return slice(128 * j, 128 * (j + 1))

    def h_dot(r0, n):
        xa = x[pl.ds(_al(r0, 16), n), :]
        y = _dot(xa, w1[...])
        m, _, rs = _stats(xa.astype(F32))
        h = _gelu(y * rs - (rs * m) * c1s[...])
        for j in range(LT):
            hbuf[j, pl.ds(_al(r0 + PAD, 8), n), :] = h[:, tile(j)]

    def k_dot(r0, n):
        kk = _dot(wkt[...], x[pl.ds(_al(r0, 16), n), :], NT)
        pk = _phi(kk[0:D, :])
        g = 0.5 * jnp.tanh(0.5 * kk[D:D + 1, :]) + 0.5
        gts[pl.ds(_al(r0, 128), n), :] = jnp.broadcast_to(g, (128, n)).T
        zs = pk[:, 0:128]
        for j in range(1, n // 128):
            zs = zs + pk[:, tile(j)]
        return pk.astype(BF16), zs

    start('x0 gw a0')
    for j in range(LT):
        hbuf[j, 0:PAD, :] = jnp.zeros((PAD, 128), F32)
        hbuf[j, PAD + S:PAD + S + PAD, :] = jnp.zeros((PAD, 128), F32)
    ones = jnp.ones((16, D), BF16)
    wait('x0')
    start('a1 x1')
    wait('gw')
    m0, _, rs0 = _stats(x[0:T0, :].astype(F32))
    st0[0] = jnp.broadcast_to(rs0, (T0, 128))
    st0[1] = jnp.broadcast_to(rs0 * m0, (T0, 128))
    wait('a0')
    start('wk x2')
    hacc[...] = _dot(jnp.concatenate([ones[:, 0:KA], x[0:T0, 0:KA]], axis=0), w1[0:KA, :])
    wait('a1')
    start('r0 wq')
    y0 = hacc[...] + _dot(jnp.concatenate([ones[:, KA:D], x[0:T0, KA:D]], axis=0), w1[KA:D, :])
    c1 = y0[0:1, :]
    c1s[...] = c1
    for j in range(LT):
        hbuf[j, PAD:PAD + T0, :] = _gelu(y0[16:16 + T0, tile(j)] * st0[0] - st0[1] * c1[:, tile(j)])
    wait('x1')
    start('r1 r2')
    h_dot(T0, T1 // 2)
    h_dot(T0 + T1 // 2, T1 // 2)
    wait('wk x2')
    start(late[0])
    for a, b in ((0, 256), (256, 512), (512, 640)):
        wkt[0:D, a:b] = wk[a:b, :].T
    row = lax.broadcasted_iota(jnp.int32, (16, D), 0)
    wkt[D:D + 16, :] = jnp.where(
        row == 0, jnp.broadcast_to(gw[...].astype(F32).reshape(1, D), (16, D)), 0.0).astype(BF16)
    h_dot(T0 + T1, T2)
    th = TK // 2
    pka, zsa = k_dot(0, th)
    pkb, zsb = k_dot(th, th)
    zacc[...] = zsa + zsb
    ga0 = _dot(pka, x[0:th, :])
    gacc[...] = ga0 + _dot(pkb, x[th:TK, :])

    def phase1(t, carry):
        x_rest(t).wait()
        r0 = _al((t + 1) * TK, 128)
        h_dot(RF + t * HR, HA)
        pk, zs = k_dot(r0, TK)
        h_dot(RF + t * HR + HA, HR - HA)
        zacc[...] += zs
        gacc[...] += _dot(pk, x[pl.ds(r0, TK), :])
        for i in range(1, NL):
            @pl.when(t == i - 1)
            def _(i=i):
                start(late[i])
        return carry

    lax.fori_loop(0, NL, phase1, 0)

    def wq_permute():
        for lt in range(LT):
            tmp_q[lt] = wq[tile(lt), :].T.astype(F32)
            for j in range(LT):
                for c in range(4):
                    wqp[lt, pl.ds(128 * j + 32 * c, 32), :] = (
                        tmp_q[lt, pl.ds(4 * j + c, 32, stride=DH), :].astype(BF16))

    def kv_dot(j):
        a, b = KV_ROWS[j]
        kv = _dot(gacc[a:b, :].astype(BF16), wv[:, tile(j)])
        rh = (lax.broadcasted_iota(jnp.int32, (b - a, 128), 0) + a) // DH
        ch = (lax.broadcasted_iota(jnp.int32, (b - a, 128), 1) + 128 * j) // DH
        return jnp.where(rh == ch, kv, 0.0).astype(BF16)

    def m_dots(kvs):
        carry = None
        for j in range(LT):
            a, b = KV_ROWS[j]
            part = _dot(kvs[j], wo[tile(j), :])
            lo = 0
            if carry is not None:
                head = part[0:32, :] + carry
                for lt in range(LT):
                    tmp_m[lt, a:a + 32, :] = head[:, tile(lt)]
                lo = 32
            hi = (b - a) - (32 if j + 1 < LT else 0)
            for lt in range(LT):
                tmp_m[lt, a + lo:a + hi, :] = part[lo:hi, tile(lt)]
            carry = part[hi:b - a, :] if j + 1 < LT else None
        for j in range(LT):
            for c in range(4):
                for lt in range(LT):
                    mp[pl.ds(128 * j + 32 * c, 32), tile(lt)] = (
                        tmp_m[lt, pl.ds(4 * j + c, 32, stride=DH), :].astype(BF16))

    def z_setup():
        for j in range(LT):
            zp = jnp.concatenate([zacc[pl.ds(4 * j + c, 32, stride=DH), :] for c in range(4)], axis=0)
            zrow[:, tile(j)] = jnp.sum(zp.T, axis=0, keepdims=True)

    def q_dot(s, r0, n):
        wt = jnp.concatenate([wqp[lt] for lt in range(LT)], axis=1)
        pqs[s, 0:n] = _phi(_dot(x[pl.ds(_al(r0, 16), n), :], wt, NT))

    def normalize(s, n):
        z = zrow[...]
        pq = pqs[s, 0:n]
        den = pq[:, tile(0)] * z[:, tile(0)]
        for j in range(1, LT):
            den = den + pq[:, tile(j)] * z[:, tile(j)]
        den = den + pltpu.roll(den, 64, 1)
        den = den + pltpu.roll(den, 32, 1)
        inv = 1.0 / (den + 1e-6)
        pqn[s, 0:n] = jnp.concatenate([pq[:, tile(j)] * inv for j in range(LT)], axis=1).astype(BF16)

    def shift(s, r0, n):
        def hl(j, sh):
            return hbuf[j, pl.ds(r0 + PAD - sh, n), :]
        lane = lax.broadcasted_iota(jnp.int32, (n, 128), 1)
        hsb[s, 0:n] = jnp.concatenate([
            hl(0, 1),
            jnp.where(lane < 32, hl(1, 1), hl(1, -1)),
            jnp.where(lane < 64, hl(2, -1), hl(2, 2)),
            jnp.where(lane < 96, hl(3, 2), hl(3, -2)),
            hl(4, -2)], axis=1).astype(BF16)

    def w2_dot(s, r0, n):
        x1s[s, 0:n] = x[pl.ds(_al(r0, 16), n), :].astype(F32) + _dot(hsb[s, 0:n], w2[...])

    def m_dot(s, r0, n):
        a = _dot(pqn[s, 0:n], mp[...])
        g = gts[pl.ds(_al(r0, 16), n), :]
        for j in range(LT):
            gas[s, 0:n, tile(j)] = g * a[:, tile(j)] + (1.0 - g) * x1s[s, 0:n, tile(j)]

    def ln2(s, n):
        _, xc, rs = _stats(x1s[s, 0:n])
        xns[s, 0:n] = (xc * rs).astype(BF16)

    def w3_dot(s, n):
        xn = xns[s, 0:n]
        gus[s, 0:n, 0:FM] = _gelu(_dot(xn, w3t[0:FM, :], NT)).astype(BF16)
        ut = _dot(w3t[FM:F, :], xn, NT)
        gus[s, 0:n, FM:F] = _gelu(ut).T.astype(BF16)

    def w4_dot(s, r0, n, i, by_cols):
        h2 = _dot(gus[s, 0:n, 0:F], w4[...])
        r0 = _al(r0, 16)
        g = gts[pl.ds(r0, n), :]
        for j in range(LT):
            ob[pl.ds(r0, n), tile(j)] = (gas[s, 0:n, tile(j)] + (1.0 - g) * h2[:, tile(j)]).astype(BF16)
            if by_cols:
                out_copy_cols(r0, n, i, j).start()
        if not by_cols:
            out_copy(r0, n, i).start()

    wait('wv w2 wo w3a w3b w4a w4b wq')
    wq_permute()
    kvs = [kv_dot(0), kv_dot(1)]
    shift(0, 0, TM)
    w2_dot(0, 0, TM)
    kvs += [kv_dot(2), kv_dot(3), kv_dot(4)]
    z_setup()
    m_dots(kvs)
    ln2(0, TM)
    w3_dot(0, TM)
    q_dot(0, 0, TM)
    normalize(0, TM)
    h2_0 = _dot(gus[0, 0:TM, 0:F], w4[...])
    g_0 = gts[0:TM, :]
    for j in range(LT):
        gas[0, 0:TM, tile(j)] = (1.0 - g_0) * (x1s[0, 0:TM, tile(j)] + h2_0[:, tile(j)])
    a_0 = _dot(pqn[0, 0:TM], mp[...])
    for j in range(LT):
        ob[0:TM, tile(j)] = (g_0 * a_0[:, tile(j)] + gas[0, 0:TM, tile(j)]).astype(BF16)
    out_copy(0, TM, 0).start()

    def phase2(t, carry):
        ra = _al(TM + t * (TA + TB), 16)
        rb = _al(ra + TA, 16)
        i0 = 1 + t * (1 + LT)
        q_dot(0, ra, TA)
        shift(0, ra, TA)
        w2_dot(0, ra, TA)
        q_dot(1, rb, TB)
        normalize(0, TA)
        shift(1, rb, TB)
        m_dot(0, ra, TA)
        w2_dot(1, rb, TB)
        ln2(0, TA)
        w3_dot(0, TA)
        normalize(1, TB)
        m_dot(1, rb, TB)
        ln2(1, TB)
        w4_dot(0, ra, TA, i0, False)
        w3_dot(1, TB)
        w4_dot(1, rb, TB, i0 + 1, True)
        return carry

    lax.fori_loop(0, N2, phase2, 0)

    out_copy(0, TM, 0).wait()
    for t in range(N2):
        ra = TM + t * (TA + TB)
        i0 = 1 + t * (1 + LT)
        out_copy(ra, TA, i0).wait()
        for j in range(LT):
            out_copy_cols(ra + TA, TB, i0 + 1, j).wait()


def _compiler_params():
    vmem = dict(vmem_limit_bytes=100 * 1024 * 1024)
    try:
        return pltpu.CompilerParams(disable_bounds_checks=True, disable_semaphore_checks=True, **vmem)
    except TypeError:
        return pltpu.CompilerParams(**vmem)


@jax.jit
def pallas_gated_mix__linear_attn_block__mixer_s_mlp__prompt_kernel(
        A_x, A_wqkv, A_wo, B_x, B_w1, B_w2, B_w3, B_w4, gate_w):
    del B_x
    hbm = pl.BlockSpec(memory_space=pltpu.MemorySpace.HBM)
    vmem = pltpu.VMEM
    return pl.pallas_call(
        _kernel,
        out_shape=jax.ShapeDtypeStruct((1, S, D), BF16),
        in_specs=[hbm] * 8,
        out_specs=hbm,
        scratch_shapes=[
            vmem((S, D), BF16),
            vmem((D, D), BF16), vmem((D, D), BF16), vmem((D, D), BF16),
            vmem((D, D), BF16), vmem((D, D), BF16), vmem((D, D), BF16),
            vmem((F, D), BF16), vmem((F, D), BF16),
            vmem((D,), BF16), vmem((S, D), BF16),
            vmem((D + 16, D), BF16),
            vmem((LT, D, 128), BF16),
            vmem((LT, D, 128), F32),
            vmem((LT, D, 128), F32),
            vmem((LT, S + 2 * PAD, 128), F32),
            vmem((D, D), F32),
            vmem((D, 128), F32),
            vmem((D, D), BF16),
            vmem((1, D), F32),
            vmem((T0 + 16, D), F32),
            vmem((2, T0, 128), F32),
            vmem((1, D), F32),
            vmem((2, TMAX, D), F32),
            vmem((2, TMAX, D), BF16),
            vmem((2, TMAX, D), BF16),
            vmem((2, TMAX, D), F32),
            vmem((2, TMAX, D), BF16),
            vmem((2, TMAX, D), F32),
            vmem((2, TMAX, F), BF16),
            vmem((S, 128), F32),
            pltpu.SemaphoreType.DMA((N_SEM,)),
        ],
        compiler_params=_compiler_params(),
        name='gm',
    )(A_x, A_wqkv, A_wo, B_w1, B_w2, B_w3.T, B_w4, gate_w)
```

```python
import jax
import jax.numpy as jnp
from jax import lax
from jax.experimental import pallas as pl
from jax.experimental.pallas import tpu as pltpu

S, D, F, H, DH = 2048, 640, 1728, 32, 20
LT = D // 128
FM = (F // 128) * 128
FH = F // 2
PAD = 8
KV_ROWS = ((0, 144), (112, 272), (240, 400), (368, 528), (496, 640))

T0 = 256
T1 = 352
KA = 256
N1 = 4
TK = S // N1
HR = 432
NL = N1 - 1
RF = S - NL * HR
T2 = RF - T0 - T1
HA = (HR // 32) * 16
TM = 256
TA, TB = 192, 256
N2 = (S - TM) // (TA + TB)
assert T2 > 0 and T2 % 16 == 0 and T1 % 32 == 0 and TM + N2 * (TA + TB) == S

F32 = jnp.float32
BF16 = jnp.bfloat16
NN = (((1,), (0,)), ((), ()))
NT = (((1,), (1,)), ((), ()))

W_A0, W_A1, W_V, W_Q, W_O, W_2, W_3A, W_3B, W_4A, W_4B, W_G, W_K = range(12)
X_0 = 12
O_0 = X_0 + 3 + NL
N_OUT = 1 + N2 * (1 + LT)
N_SEM = O_0 + N_OUT


def _dot(a, b, dims=NN):
    return lax.dot_general(a, b, dims, preferred_element_type=F32)


def _phi(t):
    return jnp.where(t > 0, t + 1.0, jnp.exp(t)) + 1e-6


def _gelu(x):
    c = 0.7978845608028654
    inner = x * (c + (c * 0.044715) * (x * x))
    hx = 0.5 * x
    return hx + hx * jnp.tanh(inner)


def _stats(x):
    m = jnp.mean(x, axis=-1, keepdims=True)
    xc = x - m
    v = jnp.mean(xc * xc, axis=-1, keepdims=True)
    return m, xc, lax.rsqrt(v + 1e-5)


def _al(r, m):
    return r if isinstance(r, int) else pl.multiple_of(r, m)


def _kernel(x_hbm, wqkv_hbm, wo_hbm, w1_hbm, w2_hbm, w3t_hbm, w4_hbm, gw_hbm, out_hbm,
            x, wq, wk, wv, wo, w1, w2, w3t, w4, gw, ob,
            wkt, wqp, tmp_m, tmp_q, hbuf, gacc, zacc, mp, zrow,
            hacc, st0, c1s, gts, sem):
    def x_copy(r0, n, i):
        return pltpu.make_async_copy(x_hbm.at[0, pl.ds(r0, n), :], x.at[pl.ds(r0, n), :], sem.at[X_0 + i])

    def x_rest(t):
        return x_copy(RF + t * HR, HR, 3 + t)

    def rows_copy(src, dst, r0, n, s):
        return pltpu.make_async_copy(src.at[pl.ds(r0, n), :], dst.at[pl.ds(r0, n), :], sem.at[s])

    copies = {
        'a0': lambda: rows_copy(w1_hbm, w1, 0, KA, W_A0),
        'a1': lambda: rows_copy(w1_hbm, w1, KA, D - KA, W_A1),
        'wv': lambda: pltpu.make_async_copy(wqkv_hbm.at[:, pl.ds(2 * D, D)], wv, sem.at[W_V]),
        'wq': lambda: pltpu.make_async_copy(wqkv_hbm.at[:, pl.ds(0, D)], wq, sem.at[W_Q]),
        'wo': lambda: pltpu.make_async_copy(wo_hbm, wo, sem.at[W_O]),
        'w2': lambda: pltpu.make_async_copy(w2_hbm, w2, sem.at[W_2]),
        'w3a': lambda: rows_copy(w3t_hbm, w3t, 0, FH, W_3A),
        'w3b': lambda: rows_copy(w3t_hbm, w3t, FH, FH, W_3B),
        'w4a': lambda: rows_copy(w4_hbm, w4, 0, FH, W_4A),
        'w4b': lambda: rows_copy(w4_hbm, w4, FH, FH, W_4B),
        'gw': lambda: pltpu.make_async_copy(gw_hbm, gw, sem.at[W_G]),
        'wk': lambda: pltpu.make_async_copy(wqkv_hbm.at[:, pl.ds(D, D)], wk, sem.at[W_K]),
        'x0': lambda: x_copy(0, T0, 0),
        'x1': lambda: x_copy(T0, T1, 1),
        'x2': lambda: x_copy(T0 + T1, T2, 2),
        'r0': lambda: x_rest(0),
        'r1': lambda: x_rest(1),
        'r2': lambda: x_rest(2),
    }

    def start(names):
        for n in names.split():
            copies[n]().start()

    def wait(names):
        for n in names.split():
            copies[n]().wait()

    late = ('wv w2', 'wo w3a', 'w3b w4a w4b')

    def out_copy(r0, n, i):
        return pltpu.make_async_copy(ob.at[pl.ds(r0, n), :], out_hbm.at[0, pl.ds(r0, n), :], sem.at[O_0 + i])

    def out_copy_cols(r0, n, i, j):
        return pltpu.make_async_copy(ob.at[pl.ds(r0, n), pl.ds(128 * j, 128)],
                                     out_hbm.at[0, pl.ds(r0, n), pl.ds(128 * j, 128)], sem.at[O_0 + i + j])

    def tile(j):
        return slice(128 * j, 128 * (j + 1))

    def h_dot(r0, n):
        xa = x[pl.ds(_al(r0, 16), n), :]
        y = _dot(xa, w1[...])
        m, _, rs = _stats(xa.astype(F32))
        h = _gelu(y * rs - (rs * m) * c1s[...])
        for j in range(LT):
            hbuf[j, pl.ds(_al(r0 + PAD, 8), n), :] = h[:, tile(j)]

    def k_dot(r0, n):
        kk = _dot(wkt[...], x[pl.ds(_al(r0, 16), n), :], NT)
        pk = _phi(kk[0:D, :])
        g = 0.5 * jnp.tanh(0.5 * kk[D:D + 1, :]) + 0.5
        gts[pl.ds(_al(r0, 128), n), :] = jnp.broadcast_to(g, (128, n)).T
        zs = pk[:, 0:128]
        for j in range(1, n // 128):
            zs = zs + pk[:, tile(j)]
        return pk.astype(BF16), zs

    start('x0 gw a0')
    for j in range(LT):
        hbuf[j, 0:PAD, :] = jnp.zeros((PAD, 128), F32)
        hbuf[j, PAD + S:PAD + S + PAD, :] = jnp.zeros((PAD, 128), F32)
    ones = jnp.ones((16, D), BF16)
    wait('x0')
    start('a1 x1')
    wait('gw')
    m0, _, rs0 = _stats(x[0:T0, :].astype(F32))
    st0[0] = jnp.broadcast_to(rs0, (T0, 128))
    st0[1] = jnp.broadcast_to(rs0 * m0, (T0, 128))
    wait('a0')
    start('wk x2')
    hacc[...] = _dot(jnp.concatenate([ones[:, 0:KA], x[0:T0, 0:KA]], axis=0), w1[0:KA, :])
    wait('a1')
    start('r0 wq')
    y0 = hacc[...] + _dot(jnp.concatenate([ones[:, KA:D], x[0:T0, KA:D]], axis=0), w1[KA:D, :])
    c1 = y0[0:1, :]
    c1s[...] = c1
    for j in range(LT):
        hbuf[j, PAD:PAD + T0, :] = _gelu(y0[16:16 + T0, tile(j)] * st0[0] - st0[1] * c1[:, tile(j)])
    wait('x1')
    start('r1 r2')
    h_dot(T0, T1 // 2)
    h_dot(T0 + T1 // 2, T1 // 2)
    wait('wk x2')
    start(late[0])
    for a, b in ((0, 256), (256, 512), (512, 640)):
        wkt[0:D, a:b] = wk[a:b, :].T
    row = lax.broadcasted_iota(jnp.int32, (16, D), 0)
    wkt[D:D + 16, :] = jnp.where(
        row == 0, jnp.broadcast_to(gw[...].astype(F32).reshape(1, D), (16, D)), 0.0).astype(BF16)
    h_dot(T0 + T1, T2)
    th = TK // 2
    pka, zsa = k_dot(0, th)
    pkb, zsb = k_dot(th, th)
    zacc[...] = zsa + zsb
    ga0 = _dot(pka, x[0:th, :])
    gacc[...] = ga0 + _dot(pkb, x[th:TK, :])

    def phase1(t, carry):
        x_rest(t).wait()
        r0 = _al((t + 1) * TK, 128)
        h_dot(RF + t * HR, HA)
        pk, zs = k_dot(r0, TK)
        h_dot(RF + t * HR + HA, HR - HA)
        zacc[...] += zs
        gacc[...] += _dot(pk, x[pl.ds(r0, TK), :])
        for i in range(1, NL):
            @pl.when(t == i - 1)
            def _(i=i):
                start(late[i])
        return carry

    lax.fori_loop(0, NL, phase1, 0)

    def wq_permute():
        for lt in range(LT):
            tmp_q[lt] = wq[tile(lt), :].T.astype(F32)
            for j in range(LT):
                for c in range(4):
                    wqp[lt, pl.ds(128 * j + 32 * c, 32), :] = (
                        tmp_q[lt, pl.ds(4 * j + c, 32, stride=DH), :].astype(BF16))

    def kv_dot(j):
        a, b = KV_ROWS[j]
        kv = _dot(gacc[a:b, :].astype(BF16), wv[:, tile(j)])
        rh = (lax.broadcasted_iota(jnp.int32, (b - a, 128), 0) + a) // DH
        ch = (lax.broadcasted_iota(jnp.int32, (b - a, 128), 1) + 128 * j) // DH
        return jnp.where(rh == ch, kv, 0.0).astype(BF16)

    def m_dots(kvs):
        carry = None
        for j in range(LT):
            a, b = KV_ROWS[j]
            part = _dot(kvs[j], wo[tile(j), :])
            lo = 0
            if carry is not None:
                head = part[0:32, :] + carry
                for lt in range(LT):
                    tmp_m[lt, a:a + 32, :] = head[:, tile(lt)]
                lo = 32
            hi = (b - a) - (32 if j + 1 < LT else 0)
            for lt in range(LT):
                tmp_m[lt, a + lo:a + hi, :] = part[lo:hi, tile(lt)]
            carry = part[hi:b - a, :] if j + 1 < LT else None
        for j in range(LT):
            for c in range(4):
                for lt in range(LT):
                    mp[pl.ds(128 * j + 32 * c, 32), tile(lt)] = (
                        tmp_m[lt, pl.ds(4 * j + c, 32, stride=DH), :].astype(BF16))

    def z_setup():
        for j in range(LT):
            zp = jnp.concatenate([zacc[pl.ds(4 * j + c, 32, stride=DH), :] for c in range(4)], axis=0)
            zrow[:, tile(j)] = jnp.sum(zp.T, axis=0, keepdims=True)

    def q_dot(r0, n):
        wt = jnp.concatenate([wqp[lt] for lt in range(LT)], axis=1)
        return _phi(_dot(x[pl.ds(_al(r0, 16), n), :], wt, NT))

    def normalize(pq):
        z = zrow[...]
        den = pq[:, tile(0)] * z[:, tile(0)]
        for j in range(1, LT):
            den = den + pq[:, tile(j)] * z[:, tile(j)]
        den = den + pltpu.roll(den, 64, 1)
        den = den + pltpu.roll(den, 32, 1)
        inv = 1.0 / (den + 1e-6)
        return jnp.concatenate([pq[:, tile(j)] * inv for j in range(LT)], axis=1).astype(BF16)

    def shift(r0, n):
        def hl(j, sh):
            return hbuf[j, pl.ds(r0 + PAD - sh, n), :]
        lane = lax.broadcasted_iota(jnp.int32, (n, 128), 1)
        return jnp.concatenate([
            hl(0, 1),
            jnp.where(lane < 32, hl(1, 1), hl(1, -1)),
            jnp.where(lane < 64, hl(2, -1), hl(2, 2)),
            jnp.where(lane < 96, hl(3, 2), hl(3, -2)),
            hl(4, -2)], axis=1).astype(BF16)

    def w2_dot(hs, r0, n):
        return x[pl.ds(_al(r0, 16), n), :].astype(F32) + _dot(hs, w2[...])

    def m_dot(pqn, x1, r0, n):
        a = _dot(pqn, mp[...])
        g = gts[pl.ds(_al(r0, 16), n), :]
        return [g * a[:, tile(j)] + (1.0 - g) * x1[:, tile(j)] for j in range(LT)]

    def ln2(x1):
        _, xc, rs = _stats(x1)
        return (xc * rs).astype(BF16)

    def w3_dot(xn):
        gu = _gelu(_dot(xn, w3t[0:FM, :], NT)).astype(BF16)
        ut = _dot(w3t[FM:F, :], xn, NT)
        return jnp.concatenate([gu, _gelu(ut).T.astype(BF16)], axis=1)

    def w4_dot(gu, ga, r0, n, i, by_cols):
        h2 = _dot(gu, w4[...])
        r0 = _al(r0, 16)
        g = gts[pl.ds(r0, n), :]
        for j in range(LT):
            ob[pl.ds(r0, n), tile(j)] = (ga[j] + (1.0 - g) * h2[:, tile(j)]).astype(BF16)
            if by_cols:
                out_copy_cols(r0, n, i, j).start()
        if not by_cols:
            out_copy(r0, n, i).start()

    wait('wv w2 wo w3a w3b w4a w4b wq')
    wq_permute()
    kvs = [kv_dot(0), kv_dot(1)]
    hs_0 = shift(0, TM)
    x1_0 = w2_dot(hs_0, 0, TM)
    kvs += [kv_dot(2), kv_dot(3), kv_dot(4)]
    z_setup()
    m_dots(kvs)
    xn_0 = ln2(x1_0)
    gu_0 = w3_dot(xn_0)
    pqn_0 = normalize(q_dot(0, TM))
    h2_0 = _dot(gu_0, w4[...])
    g_0 = gts[0:TM, :]
    b_0 = [(1.0 - g_0) * (x1_0[:, tile(j)] + h2_0[:, tile(j)]) for j in range(LT)]
    a_0 = _dot(pqn_0, mp[...])
    for j in range(LT):
        ob[0:TM, tile(j)] = (g_0 * a_0[:, tile(j)] + b_0[j]).astype(BF16)
    out_copy(0, TM, 0).start()

    def phase2(t, carry):
        ra = _al(TM + t * (TA + TB), 16)
        rb = _al(ra + TA, 16)
        i0 = 1 + t * (1 + LT)
        pq_a = q_dot(ra, TA)
        hs_a = shift(ra, TA)
        x1_a = w2_dot(hs_a, ra, TA)
        pq_b = q_dot(rb, TB)
        pqn_a = normalize(pq_a)
        hs_b = shift(rb, TB)
        ga_a = m_dot(pqn_a, x1_a, ra, TA)
        x1_b = w2_dot(hs_b, rb, TB)
        xn_a = ln2(x1_a)
        gu_a = w3_dot(xn_a)
        pqn_b = normalize(pq_b)
        ga_b = m_dot(pqn_b, x1_b, rb, TB)
        xn_b = ln2(x1_b)
        w4_dot(gu_a, ga_a, ra, TA, i0, False)
        gu_b = w3_dot(xn_b)
        w4_dot(gu_b, ga_b, rb, TB, i0 + 1, True)
        return carry

    lax.fori_loop(0, N2, phase2, 0)

    out_copy(0, TM, 0).wait()
    for t in range(N2):
        ra = TM + t * (TA + TB)
        i0 = 1 + t * (1 + LT)
        out_copy(ra, TA, i0).wait()
        for j in range(LT):
            out_copy_cols(ra + TA, TB, i0 + 1, j).wait()


def _compiler_params():
    vmem = dict(vmem_limit_bytes=100 * 1024 * 1024)
    try:
        return pltpu.CompilerParams(disable_bounds_checks=True, disable_semaphore_checks=True, **vmem)
    except TypeError:
        return pltpu.CompilerParams(**vmem)


@jax.jit
def pallas_gated_mix__linear_attn_block__mixer_s_mlp__prompt_kernel(
        A_x, A_wqkv, A_wo, B_x, B_w1, B_w2, B_w3, B_w4, gate_w):
    del B_x
    hbm = pl.BlockSpec(memory_space=pltpu.MemorySpace.HBM)
    vmem = pltpu.VMEM
    return pl.pallas_call(
        _kernel,
        out_shape=jax.ShapeDtypeStruct((1, S, D), BF16),
        in_specs=[hbm] * 8,
        out_specs=hbm,
        scratch_shapes=[
            vmem((S, D), BF16),
            vmem((D, D), BF16), vmem((D, D), BF16), vmem((D, D), BF16),
            vmem((D, D), BF16), vmem((D, D), BF16), vmem((D, D), BF16),
            vmem((F, D), BF16), vmem((F, D), BF16),
            vmem((D,), BF16), vmem((S, D), BF16),
            vmem((D + 16, D), BF16),
            vmem((LT, D, 128), BF16),
            vmem((LT, D, 128), F32),
            vmem((LT, D, 128), F32),
            vmem((LT, S + 2 * PAD, 128), F32),
            vmem((D, D), F32),
            vmem((D, 128), F32),
            vmem((D, D), BF16),
            vmem((1, D), F32),
            vmem((T0 + 16, D), F32),
            vmem((2, T0, 128), F32),
            vmem((1, D), F32),
            vmem((S, 128), F32),
            pltpu.SemaphoreType.DMA((N_SEM,)),
        ],
        compiler_params=_compiler_params(),
        name='gm',
    )(A_x, A_wqkv, A_wo, B_w1, B_w2, B_w3.T, B_w4, gate_w)
```
